```python
import os as _os
_os.environ.setdefault("JAX_PLATFORMS", "cpu")
import jax
import jax.numpy as jnp

def _softmax(x, axis=-1):
    return jax.nn.softmax(x, axis=axis)
def _gelu(x):
    return jax.nn.gelu(x, approximate=True)
def _silu(x):
    return jax.nn.silu(x)
def _sigmoid(x):
    return jax.nn.sigmoid(x)
def _layernorm(x, axis=-1, eps=1e-5):
    m = jnp.mean(x, axis=axis, keepdims=True)
    v = jnp.var(x, axis=axis, keepdims=True)
    return (x - m) / jnp.sqrt(v + eps)
def _scatter_add(tgt, idx, src, axis=0):
    return tgt.at[idx].add(src)
def _segment_sum(src, seg, n):
    return jax.ops.segment_sum(src, seg, n)
class _Rng:
    def __init__(self, key):
        self._k = key
    def _next(self):
        self._k, sub = jax.random.split(self._k)
        return sub
    def normal(self, shape):
        return jax.random.normal(self._next(), shape, dtype=jnp.bfloat16)
    def randint(self, lo, hi, shape):
        return jax.random.randint(self._next(), shape, lo, hi, dtype=jnp.int32)
    def uniform(self, shape, lo=0.0, hi=1.0):
        return jax.random.uniform(self._next(), shape, jnp.bfloat16, lo, hi)
    def permutation(self, n):
        return jax.random.permutation(self._next(), n)


kernel_name = 'concat_heads__sliding_block__ssm_conv_s4__prompt'

def setup_inputs():
    _rng = _Rng(jax.random.key(int.from_bytes(__import__("os").urandom(4), "little")))
    _w = (lambda a: (lambda t: t.astype(jnp.bfloat16) if jnp.issubdtype(t.dtype, jnp.floating) else t)(jnp.asarray(a)))
    def _A_setup():
        B, S, D = 1, 2048, 512
        return {
            "x": _w((lambda *s: _rng.normal(s) * 0.2)(B, S, D)),
            "wqkv": _w((lambda *s: _rng.normal(s) * 0.2)(D, 3 * D)),
            "wo": _w((lambda *s: _rng.normal(s) * 0.05)(D, D)),
        }
    _A_in = _A_setup()

    def _B_setup():
        B, L, D, N = 1, 2048, 512, 128
        A_re = -jnp.exp((lambda *s: _rng.normal(s) * 0.8)(D, N))
        A_im = jnp.pi * (lambda *s: _rng.normal(s) * 0.8)(D, N)
        B_re = (lambda *s: _rng.normal(s) * 0.8)(D, N)
        B_im = (lambda *s: _rng.normal(s) * 0.8)(D, N)
        C_re = (lambda *s: _rng.normal(s) * 0.8)(D, N)
        C_im = (lambda *s: _rng.normal(s) * 0.8)(D, N)
        log_dt = (lambda *s: _rng.normal(s) * 0.8)(D) * 0.5 - 4.0
        Dskip = (lambda *s: _rng.normal(s) * 0.05)(D)
        return {
            "u": _w((lambda *s: _rng.normal(s) * 0.05)(B, L, D)),
            "A_re": _w(A_re),
            "A_im": _w(A_im),
            "B_re": _w(B_re),
            "B_im": _w(B_im),
            "C_re": _w(C_re),
            "C_im": _w(C_im),
            "log_dt": _w(log_dt),
            "Dskip": _w(Dskip),
        }
    _B_in = _B_setup()

    return {
        "A_x": _A_in["x"],
        "A_wqkv": _A_in["wqkv"],
        "A_wo": _A_in["wo"],
        "B_u": _B_in["u"],
        "B_A_re": _B_in["A_re"],
        "B_A_im": _B_in["A_im"],
        "B_B_re": _B_in["B_re"],
        "B_B_im": _B_in["B_im"],
        "B_C_re": _B_in["C_re"],
        "B_C_im": _B_in["C_im"],
        "B_log_dt": _B_in["log_dt"],
        "B_Dskip": _B_in["Dskip"],
    }

def reference(A_x, A_wqkv, A_wo, B_u, B_A_re, B_A_im, B_B_re, B_B_im, B_C_re, B_C_im, B_log_dt, B_Dskip):
    def _A_ref(x, wqkv, wo):
        B, S, D = x.shape
        H = 32; Dh = D // H; W = 256
        qkv = (lambda x, *d: x.transpose(*d))((x @ wqkv).reshape(B, S, 3, H, Dh), 2, 0, 3, 1, 4)
        q, k, v = qkv[0], qkv[1], qkv[2]
        scores = jnp.einsum("bhqd,bhkd->bhqk", q, k) * (Dh ** -0.5)
        idx = jnp.arange(S)
        mask = (idx[:, None] - idx[None, :] >= 0) & (idx[:, None] - idx[None, :] < W)
        scores = jnp.where(mask[None, None], scores, -1e9)
        p = _softmax(scores, axis=-1)
        o = jnp.einsum("bhqk,bhkd->bhqd", p, v)
        return (lambda x, *d: x.transpose(*d))(o, 0, 2, 1, 3).reshape(B, S, D) @ wo

    def _B_ref(u, A_re, A_im, B_re, B_im, C_re, C_im, log_dt, Dskip):
        Bsz, L, D = u.shape
        dt = jnp.exp(log_dt)[:, None]
        A = A_re + 1j * A_im
        Bc = B_re + 1j * B_im
        Cc = C_re + 1j * C_im
        logdA = dt * A
        dB = dt * Bc
        l = (lambda x, dt: x.astype(dt))(jnp.arange(L), A_re.dtype)
        P = jnp.exp(logdA[:, :, None] * l[None, None, :])
        K = jnp.einsum("dn,dnl,dn->dl", Cc, P, dB).real
        L2 = 2 * L
        Kp = jnp.pad(K, ((0, 0), (0, L)))
        up = (lambda x, *d: x.transpose(*d))(u, 0, 2, 1)
        up = jnp.pad(up, ((0, 0), (0, 0), (0, L)))
        Kf = (lambda x, axes=(-2,-1): jnp.fft.rfft2(x.astype(jnp.float32), axes=axes))(Kp[:, None, :], axes=(-2, -1))
        Uf = (lambda x, axes=(-2,-1): jnp.fft.rfft2(x.astype(jnp.float32), axes=axes))(up[:, :, None, :], axes=(-2, -1))
        Yf = Uf * Kf[None, :, :, :]
        y = (lambda x, s, axes=(-2,-1): jnp.fft.irfft2(x, s=s, axes=axes).astype(jnp.bfloat16))(Yf, (1, L2), axes=(-2, -1))[:, :, 0, :L]
        y = (lambda x, *d: x.transpose(*d))(y, 0, 2, 1) + u * Dskip[None, None, :]
        return y

    a = _A_ref(A_x, A_wqkv, A_wo)
    b = _B_ref(B_u, B_A_re, B_A_im, B_B_re, B_B_im, B_C_re, B_C_im, B_log_dt, B_Dskip)
    return jnp.concatenate([a, b], axis=-1)
```

```python
import functools

import jax
import jax.numpy as jnp
import numpy as np
from jax import lax
from jax.experimental import pallas as pl
from jax.experimental.pallas import tpu as pltpu

f32, bf16 = jnp.float32, jnp.bfloat16
NT = (((1,), (1,)), ((), ()))
NN = (((1,), (0,)), ((), ()))

S_, D_, H_ = 2048, 512, 32
L_, N_ = 2048, 128
NF = 4096
C2 = float(0.25 * np.log2(np.e))
NEG = -1e30
GS = 4
VP, UP, FP = 33, 25, 129
NA = 24
TR = NA * 32


def _bf16_round(x):
    x = np.ascontiguousarray(x, dtype=np.float32)
    u = x.view(np.uint32).astype(np.uint64)
    r = ((u + 0x7FFF + ((u >> 16) & 1)) & 0xFFFF0000).astype(np.uint32)
    return r.view(np.float32)


LB = _bf16_round(np.arange(L_, dtype=np.float32)).astype(np.int64)
ALPHAS = list(range(8)) + [256 * m for m in range(1, 9)] + [258, 260, 262, 516, 772]
AIDX = {a: i for i, a in enumerate(ALPHAS)}


def _t_row(t):
    if t < 256:
        return AIDX[t % 8] * 32 + t // 8
    blk = t // 256
    rem = t - 256 * blk
    return AIDX[256 * blk + rem % 8] * 32 + rem // 8


def _build_consts():
    k1 = np.arange(8)
    A1 = np.zeros((16, 256, 128))
    for g in range(16):
        for n1 in range(8):
            for r in range(16):
                th = 2 * np.pi * (k1 + 0.5) * (256 * n1 + 16 * g + r) / NF
                A1[g, k1 * 32 + r, n1 * 16 + r] = np.cos(th)
                A1[g, k1 * 32 + 16 + r, n1 * 16 + r] = -np.sin(th)
    n2 = np.arange(64)
    k2 = np.arange(64)
    F2 = np.zeros((12, 128, 128))
    perm = np.array([8 * r + a for a in range(8) for r in range(8)])
    for q in range(4):
        ang = -2 * np.pi * (k2[:, None] * n2[None, :] / 64 + q * n2[None, :] / 256)
        Fr, Fi = np.cos(ang), np.sin(ang)
        F2[q] = np.block([[Fr, -Fi], [Fi, Fr]])
        F2[4 + q] = np.block([[Fr[:, perm], -Fi[:, perm]], [Fi[:, perm], Fr[:, perm]]])
        Gr, Gi = Fr.T, -Fi.T
        F2[8 + q] = np.block([[Gr, -Gi], [Gi, Gr]])
    AK = np.zeros((32, 128, 128))
    tiles = []
    for i in range(4):
        for a in range(8):
            starts = []
            for blk in range(8):
                rows = [_t_row(int(LB[256 * blk + 8 * (8 * i + r) + a])) for r in range(8)]
                todo = set(range(8))
                while todo:
                    r0 = min(todo)
                    if all(rows[r] == rows[r0] - r0 + r for r in todo):
                        st = rows[r0] - r0
                    else:
                        st = min(rows[r] for r in todo)
                    v = len(starts)
                    starts.append(st)
                    for r in sorted(todo):
                        if st <= rows[r] < st + 8:
                            th = 2 * np.pi * (k1 + 0.5) * (256 * blk + 8 * (8 * i + r) + a) / NF
                            AK[i * 8 + a, k1 * 16 + r, v * 8 + rows[r] - st] += np.cos(th)
                            AK[i * 8 + a, k1 * 16 + 8 + r, v * 8 + rows[r] - st] += -np.sin(th)
                            todo.discard(r)
            tiles.append(starts)
    AI = np.zeros((32, 64, 128))
    for g8 in range(32):
        for n1 in range(8):
            for r in range(8):
                th = 2 * np.pi * (k1 + 0.5) * (256 * n1 + 8 * g8 + r) / NF
                AI[g8, n1 * 8 + r, k1 * 16 + r] = np.cos(th) * (2.0 / NF)
                AI[g8, n1 * 8 + r, k1 * 16 + 8 + r] = -np.sin(th) * (2.0 / NF)
    cast = lambda x: np.asarray(x, dtype=np.float32).astype(bf16)
    return cast(A1), cast(AK), cast(F2), cast(AI), tiles


C_A1, C_AK, C_F2, C_AI, KT = _build_consts()
L_HI = float(np.array([0x3FB8AA00], dtype=np.uint32).view(np.float32)[0])
L_LO = float(1.4426950408889634 - L_HI)


def al(x, m):
    return x if isinstance(x, int) else pl.multiple_of(x, m)


def cmul(a, b):
    return (a[0] * b[0] - a[1] * b[1], a[0] * b[1] + a[1] * b[0])


def csq(a):
    return ((a[0] - a[1]) * (a[0] + a[1]), 2.0 * a[0] * a[1])


def sincos(x):
    kf = jnp.floor(x * 0.6366197723675814 + 0.5)
    r = ((x - kf * 1.5703125) - kf * 4.837512969970703125e-4) - kf * 7.54978995489188216e-8
    z = r * r
    s = ((-1.9515295891e-4 * z + 8.3321608736e-3) * z - 1.6666654611e-1) * z * r + r
    c = ((2.443315711809948e-5 * z - 1.388731625493765e-3) * z + 4.166664568298827e-2) * z * z - 0.5 * z + 1.0
    k = kf.astype(jnp.int32)
    swap = (k & 1) == 1
    s2 = jnp.where(swap, c, s)
    c2 = jnp.where(swap, s, c)
    s3 = jnp.where((k & 2) == 2, -s2, s2)
    c3 = jnp.where(((k + 1) & 2) == 2, -c2, c2)
    return s3, c3


def cexp(a, ph):
    e = jnp.exp(a)
    s, c = sincos(ph)
    return (e * c, e * s)


def fwd4(z):
    a0 = (z[0][0] + z[2][0], z[0][1] + z[2][1])
    a1 = (z[0][0] - z[2][0], z[0][1] - z[2][1])
    b0 = (z[1][0] + z[3][0], z[1][1] + z[3][1])
    b1 = (z[1][0] - z[3][0], z[1][1] - z[3][1])
    return [(a0[0] + b0[0], a0[1] + b0[1]), (a1[0] + b1[1], a1[1] - b1[0]),
            (a0[0] - b0[0], a0[1] - b0[1]), (a1[0] - b1[1], a1[1] + b1[0])]


def inv4(w):
    a0 = (w[0][0] + w[2][0], w[0][1] + w[2][1])
    a1 = (w[0][0] - w[2][0], w[0][1] - w[2][1])
    b0 = (w[1][0] + w[3][0], w[1][1] + w[3][1])
    b1 = (w[1][0] - w[3][0], w[1][1] - w[3][1])
    return [(a0[0] + b0[0], a0[1] + b0[1]), (a1[0] - b1[1], a1[1] + b1[0]),
            (a0[0] - b0[0], a0[1] - b0[1]), (a1[0] + b1[1], a1[1] - b1[0])]


def emit_dt(ldt_ref, dt_s):
    x = ldt_ref[...].astype(f32).reshape(1, D_)
    e = jnp.exp2(x * L_HI)
    e = e + e * ((x * L_LO) * 0.6931471805599453)
    dt = e.astype(bf16).astype(f32)
    for c in range(4):
        dt_s[c * 128:(c + 1) * 128, :] = jnp.broadcast_to(dt[:, c * 128:(c + 1) * 128], (128, 128)).T


def emit_pow(r0, RB, prm, dt_s, Ut, Vt):
    are_ref, aim_ref, bre_ref, bim_ref, cre_ref, cim_ref = prm
    sl = pl.ds(r0, RB)
    dtb = dt_s[sl, :]
    a = dtb * are_ref[sl, :].astype(f32)
    ph = dtb * aim_ref[sl, :].astype(f32)
    w = cmul((cre_ref[sl, :].astype(f32), cim_ref[sl, :].astype(f32)),
             (dtb * bre_ref[sl, :].astype(f32), dtb * bim_ref[sl, :].astype(f32)))
    l1 = cexp(a, ph)
    l256 = cexp(a * 256.0, ph * 256.0)
    l2 = csq(l1)
    l4 = csq(l2)
    l8 = csq(l4)
    V = {0: (jnp.ones_like(a), jnp.zeros_like(a)), 1: (l8[0], -l8[1])}
    for b in range(2, 32):
        V[b] = csq(V[b // 2]) if b % 2 == 0 else cmul(V[b - 1], V[1])
    for b in range(32):
        for ri in range(2):
            Vt[ri][pl.ds(r0 * VP + b, RB, stride=VP), :] = V[b][ri]
    U = {0: w}
    for a_ in range(1, 8):
        U[a_] = cmul(U[a_ - 1], l1)
    for m in range(1, 9):
        U[256 * m] = cmul(U[256 * (m - 1)], l256)
    U[258] = cmul(U[256], l2)
    U[260] = cmul(U[256], l4)
    U[262] = cmul(U[260], l2)
    U[516] = cmul(U[512], l4)
    U[772] = cmul(U[768], l4)
    for idx in range(24):
        for ri in range(2):
            val = U[ALPHAS[idx]][ri] if idx < len(ALPHAS) else jnp.zeros_like(a)
            Ut[ri][pl.ds(r0 * UP + idx, RB, stride=UP), :] = val


def emit_kgen(g, Ut, Vt, Fs):
    lane = lax.broadcasted_iota(jnp.int32, (24, 128), 1)
    Lm = jnp.concatenate([jnp.concatenate([Ut[ri][pl.ds((128 * c + g) * UP, 24), :] for c in range(4)], axis=0)
                          for ri in range(2)], axis=1)
    Rm = jnp.concatenate([jnp.concatenate([Vt[ri][pl.ds((128 * c + g) * VP, 32), :] for c in range(4)], axis=0)
                          for ri in range(2)], axis=1)
    out = lax.dot_general(Lm, Rm, NT, preferred_element_type=f32)
    F = jnp.where(lane < 64, jnp.where(lane < 32, out[0:24], out[24:48]),
                  jnp.where(lane < 96, out[48:72], out[72:96]))
    Fs[pl.ds(g, 24, stride=FP), :] = F


def emit_ttrans(idx, Fs, Ts):
    At = Fs[pl.ds(idx * FP, 128), :].T
    for c in range(4):
        Ts[pl.ds(al(c * TR + idx * 32, 8), 32), :] = At[32 * c:32 * c + 32]


def emit_f1u(gq, c, u_ref, A1_ref, Yu):
    ls = pl.ds(128 * c, 128)
    zs = []
    for j in range(4):
        g = gq + 4 * j
        tile = jnp.concatenate([u_ref[pl.ds(al(256 * n1 + 16 * g, 16), 16), ls] for n1 in range(8)], axis=0)
        zs.append(jnp.dot(A1_ref[g], tile, preferred_element_type=f32))
    for k1 in range(8):
        y = fwd4([(zs[j][32 * k1:32 * k1 + 16], zs[j][32 * k1 + 16:32 * k1 + 32]) for j in range(4)])
        for q in range(4):
            for ri in range(2):
                Yu[q * 8 + k1, pl.ds(al(ri * 64 + 16 * gq, 16), 16), ls] = y[q][ri].astype(bf16)


def emit_f1k(a2, c, Ts, AK_ref, Yk):
    zs = [[None, None] for _ in range(4)]
    for aa in range(2):
        a = 2 * a2 + aa
        for i in range(4):
            st = KT[i * 8 + a]
            tile = jnp.concatenate([Ts[pl.ds(c * TR + s0, 8), :] for s0 in st], axis=0)
            zs[i][aa] = jnp.dot(AK_ref[i * 8 + a, :, 0:8 * len(st)], tile, preferred_element_type=f32)
    for k1 in range(8):
        zz = []
        for i in range(4):
            re = jnp.concatenate([zs[i][aa][16 * k1:16 * k1 + 8] for aa in range(2)], axis=0)
            im = jnp.concatenate([zs[i][aa][16 * k1 + 8:16 * k1 + 16] for aa in range(2)], axis=0)
            zz.append((re, im))
        y = fwd4(zz)
        for q in range(4):
            for ri in range(2):
                Yk[q * 8 + k1, c, pl.ds(ri * 64 + 16 * a2, 16), :] = y[q][ri].astype(bf16)


def emit_f2(k1s, Yu, Yk, F2_ref, Pb, Zs):
    LAG = 3
    R = Pb.shape[0]
    items = [(k1, c, q) for k1 in k1s for c in range(4) for q in (0, 2, 1, 3)]

    def X(i):
        k1, c, q = items[i]
        Uh = jnp.dot(F2_ref[q], Yu[q * 8 + k1, :, pl.ds(128 * c, 128)], preferred_element_type=f32)
        Kh = jnp.dot(F2_ref[4 + q], Yk[q * 8 + k1, c], preferred_element_type=f32)
        Pr = Uh[0:64] * Kh[0:64] - Uh[64:128] * Kh[64:128]
        Pi = Uh[0:64] * Kh[64:128] + Uh[64:128] * Kh[0:64]
        Pb[i % R] = jnp.concatenate([Pr, Pi], axis=0).astype(bf16)

    ws = {}

    def Y(i):
        k1, c, q = items[i]
        W = jnp.dot(F2_ref[8 + q], Pb[i % R], preferred_element_type=f32)
        ws[q] = (W[0:64], W[64:128])
        if q == 3:
            z = inv4([ws[0], ws[1], ws[2], ws[3]])
            for j in range(4):
                for ri in range(2):
                    for b8 in range(8):
                        Zs[8 * j + b8, c, pl.ds(al(k1 * 16 + ri * 8, 8), 8), :] = z[j][ri][8 * b8:8 * b8 + 8]

    n = len(items)
    for i in range(min(LAG, n)):
        X(i)
    for i in range(n):
        if i + LAG < n:
            X(i + LAG)
        Y(i)


def emit_i1(g16, c, u_ref, dsk, AI_ref, Zs, b_s):
    ls = pl.ds(128 * c, 128)
    ys = [jnp.dot(AI_ref[2 * g16 + h], Zs[2 * g16 + h, c], preferred_element_type=f32) for h in range(2)]
    dk = dsk[:, 128 * c:128 * c + 128]
    for n1 in range(8):
        y = jnp.concatenate([ys[0][8 * n1:8 * n1 + 8], ys[1][8 * n1:8 * n1 + 8]], axis=0)
        rows = pl.ds(al(256 * n1 + 16 * g16, 16), 16)
        ub = u_ref[rows, ls].astype(f32)
        yb = y.astype(bf16).astype(f32)
        sk = (ub * dk).astype(bf16).astype(f32)
        b_s[rows, ls] = (yb + sk).astype(bf16)


def emit_proj(r0, TB, x_ref, wqkv_ref, wqT, wvT, qt_s, k_s, vt_s):
    xb = x_ref[pl.ds(r0, TB), :]
    k_s[pl.ds(r0, TB), :] = jnp.dot(xb, wqkv_ref[:, 512:1024], preferred_element_type=f32).astype(bf16)
    qt_s[:, pl.ds(r0, TB)] = lax.dot_general(wqT[...], xb, NT, preferred_element_type=f32).astype(bf16)
    vt_s[:, pl.ds(r0, TB)] = lax.dot_general(wvT[...], xb, NT, preferred_element_type=f32).astype(bf16)


def emit_attention(qt_s, k_s, vt_s, wo_ref, a_s, oT_a, oT_b, s_a, s_b, m_a, m_b, after_outproj):
    row = lax.broadcasted_iota(jnp.int32, (128, 128), 0)
    col = lax.broadcasted_iota(jnp.int32, (128, 128), 1)
    near_ok = row <= col
    z16 = jnp.zeros((16, 128), bf16)

    def qk_group(qb, nt, g, s_ref, m_ref):
        q0 = al(qb * 128, 128)
        k0 = al(q0 - (nt - 1) * 128, 128)
        hg = (g * GS) // 8
        ls = pl.ds(hg * 128, 128)
        if nt == 3:
            pcs = []
            for i in range(8):
                pcs.append(k_s[pl.ds(al(k0 + 16 * i, 16), 16), ls])
                pcs.append(k_s[pl.ds(al(k0 + 256 + 16 * i, 16), 16), ls])
            pcs.append(k_s[pl.ds(al(k0 + 128, 128), 128), ls])
            Kw = jnp.concatenate(pcs, axis=0)
        else:
            Kw = k_s[pl.ds(k0, nt * 128), ls]
        for hh in range(GS):
            h = g * GS + hh
            hl = h % 8
            qt = qt_s[pl.ds(h * 16, 16), pl.ds(q0, 128)]
            W = jnp.concatenate([z16] * hl + [qt] + [z16] * (7 - hl), axis=0)
            ST = lax.dot_general(Kw, W, NN, preferred_element_type=f32)
            if nt == 3:
                mg = []
                for i in range(8):
                    far = ST[32 * i:32 * i + 16]
                    near = ST[32 * i + 16:32 * i + 32]
                    mg.append(jnp.where(near_ok[16 * i:16 * i + 16], near, far))
                mrg = jnp.concatenate(mg, axis=0)
                mid = ST[256:384]
                s_ref[hh, 0:128] = mrg
                s_ref[hh, 128:256] = mid
                m = jnp.max(jnp.maximum(mrg, mid), axis=0, keepdims=True)
            elif nt == 2:
                mid, near = ST[0:128], ST[128:256]
                mrg = jnp.where(near_ok, near, NEG)
                s_ref[hh, 0:128] = mrg
                s_ref[hh, 128:256] = mid
                m = jnp.max(jnp.maximum(mrg, mid), axis=0, keepdims=True)
            else:
                mrg = jnp.where(near_ok, ST, NEG)
                s_ref[hh, 0:128] = mrg
                m = jnp.max(mrg, axis=0, keepdims=True)
            m_ref[hh] = jnp.broadcast_to(m, (8, 128))

    def pv_group(qb, nt, g, s_ref, m_ref, oT_s):
        q0 = al(qb * 128, 128)
        k0 = al(q0 - (nt - 1) * 128, 128)
        for hh in range(GS):
            h = g * GS + hh
            m8 = m_ref[hh]
            m = jnp.concatenate([m8] * 16, axis=0)
            pm = jnp.exp2((s_ref[hh, 0:128] - m) * C2)
            den8 = pm[0:8]
            for i in range(1, 16):
                den8 = den8 + pm[8 * i:8 * i + 8]
            vt = vt_s[pl.ds(h * 16, 16), pl.ds(k0, nt * 128)]
            if nt == 3:
                O1 = lax.dot_general(vt[:, 0:128], jnp.where(near_ok, 0.0, pm), NN, preferred_element_type=f32)
                O2 = lax.dot_general(vt[:, 256:384], jnp.where(near_ok, pm, 0.0), NN, preferred_element_type=f32)
            if nt >= 2:
                pd = jnp.exp2((s_ref[hh, 128:256] - m) * C2)
                for i in range(16):
                    den8 = den8 + pd[8 * i:8 * i + 8]
            if nt == 3:
                O3 = lax.dot_general(vt[:, 128:256], pd, NN, preferred_element_type=f32)
                OT = O1 + O2 + O3
            elif nt == 2:
                OT = (lax.dot_general(vt[:, 128:256], pm, NN, preferred_element_type=f32)
                      + lax.dot_general(vt[:, 0:128], pd, NN, preferred_element_type=f32))
            else:
                OT = lax.dot_general(vt, pm, NN, preferred_element_type=f32)
            den = jnp.sum(den8, axis=0, keepdims=True)
            o = OT * (1.0 / den)
            oT_s[pl.ds(h * 16, 16), :] = o.astype(bf16)

    def outproj(qb, oT_s):
        q0 = al(qb * 128, 128)
        o = oT_s[...].T
        a_s[pl.ds(q0, 128), :] = jnp.dot(o, wo_ref[...], preferred_element_type=f32).astype(bf16)
        after_outproj(qb)

    NG = H_ // GS
    bufs = [(s_a, m_a), (s_b, m_b)]
    OPG = 2

    def qblock(qb, nt, nt_next, oT_cur, oT_prev, prev_qb, nxt_qb):
        for g in range(NG):
            if g + 1 < NG:
                qk_group(qb, nt, g + 1, *bufs[(g + 1) % 2])
            elif nt_next is not None:
                qk_group(nxt_qb, nt_next, 0, *bufs[0])
            pv_group(qb, nt, g, *bufs[g % 2], oT_cur)
            if g == OPG and prev_qb is not None:
                outproj(prev_qb, oT_prev)

    qk_group(0, 1, 0, *bufs[0])
    qblock(0, 1, 2, oT_a, oT_b, None, 1)
    qblock(1, 2, 3, oT_b, oT_a, 0, 2)

    def body(i, c):
        qb = 2 + 2 * i
        qblock(qb, 3, 3, oT_a, oT_b, qb - 1, qb + 1)
        qblock(qb + 1, 3, 3, oT_b, oT_a, qb, jnp.minimum(qb + 2, 15))
        return c

    lax.fori_loop(0, 7, body, 0)
    outproj(15, oT_b)


def kernel(x_h, wqkv_h, wo_h, u_h, are_h, aim_h, bre_h, bim_h, cre_h, cim_h, ldt_h, dsk_h,
           A1_h, AK_h, F2_h, AI_h,
           o_h,
           x_ref, wqkv_ref, wo_ref, u_ref, are, aim, bre, bim, cre, cim, ldt_ref, dsk_ref,
           A1_ref, AK_ref, F2_ref, AI_ref,
           qt_s, k_s, vt_s, wqT, wvT, oT_a, oT_b, s_a, s_b, m_a, m_b, a_s, b_s,
           dt_s, Utr, Uti, Vtr, Vti, Fs, Ts, Yu, Yk, Pb, Zs,
           sem_in, sem_out):
    Ut = (Utr, Uti)
    Vt = (Vtr, Vti)
    prm = (are, aim, bre, bim, cre, cim)
    TB = 256
    NB = S_ // TB
    order = [(ldt_h, ldt_ref), (wqkv_h, wqkv_ref)]
    cps = {}
    idx = 0

    def mk(name, src, dst):
        nonlocal idx
        cp = pltpu.make_async_copy(src, dst, sem_in.at[idx])
        idx += 1
        cp.start()
        cps[name] = cp

    mk("ldt", ldt_h, ldt_ref)
    mk("wqkv", wqkv_h, wqkv_ref)
    for i, (s, d) in enumerate(zip((are_h, aim_h, bre_h, bim_h, cre_h, cim_h), prm)):
        mk("p%d" % i, s, d)
    for i in range(NB):
        mk("x%d" % i, x_h.at[pl.ds(i * TB, TB), :], x_ref.at[pl.ds(i * TB, TB), :])
    mk("u", u_h, u_ref)
    mk("A1", A1_h, A1_ref)
    mk("AK", AK_h, AK_ref)
    mk("F2", F2_h, F2_ref)
    mk("AI", AI_h, AI_ref)
    mk("dsk", dsk_h, dsk_ref)
    mk("wo", wo_h, wo_ref)

    cps["ldt"].wait()
    emit_dt(ldt_ref, dt_s)
    cps["wqkv"].wait()
    wqT[...] = wqkv_ref[:, 0:512].T
    wvT[...] = wqkv_ref[:, 1024:1536].T
    for i in range(6):
        cps["p%d" % i].wait()

    def proj_body(i, c):
        r0 = pl.multiple_of(i * TB, TB)
        pltpu.make_async_copy(x_h.at[pl.ds(r0, TB), :], x_ref.at[pl.ds(r0, TB), :], sem_in.at[8 + i]).wait()
        emit_proj(r0, TB, x_ref, wqkv_ref, wqT, wvT, qt_s, k_s, vt_s)
        for s in range(4):
            emit_pow(pl.multiple_of(i * 64 + s * 16, 16), 16, prm, dt_s, Ut, Vt)
        return c

    lax.fori_loop(0, NB, proj_body, 0)

    GU = 32

    def kgen_body(i, c):
        for gg in range(GU):
            emit_kgen(i * GU + gg, Ut, Vt, Fs)
        return c

    lax.fori_loop(0, 128 // GU, kgen_body, 0)

    cps["u"].wait()
    cps["A1"].wait()

    def f1u_body(gq, c):
        for cc in range(4):
            emit_f1u(gq, cc, u_ref, A1_ref, Yu)
        for t in range(6):
            emit_ttrans(gq * 6 + t, Fs, Ts)
        return c

    lax.fori_loop(0, 4, f1u_body, 0)

    cps["AK"].wait()

    def f1k_body(cc, c):
        for a2 in range(4):
            emit_f1k(a2, cc, Ts, AK_ref, Yk)
        return c

    lax.fori_loop(0, 4, f1k_body, 0)

    cps["F2"].wait()
    F2U = 2

    def f2_body(i, c):
        emit_f2([i * F2U + t for t in range(F2U)], Yu, Yk, F2_ref, Pb, Zs)
        return c

    lax.fori_loop(0, 8 // F2U, f2_body, 0)

    cps["AI"].wait()
    cps["dsk"].wait()
    dsk = dsk_ref[...].astype(f32).reshape(1, D_)
    IU = 4

    def i1_body(i, c):
        for t in range(IU):
            for cc in range(4):
                emit_i1(i * IU + t, cc, u_ref, dsk, AI_ref, Zs, b_s)
        return c

    lax.fori_loop(0, 16 // IU, i1_body, 0)
    cp_b = pltpu.make_async_copy(b_s, o_h.at[:, pl.ds(512, 512)], sem_out.at[16])
    cp_b.start()

    cps["wo"].wait()

    def out_cp(qb):
        q0 = al(qb * 128, 128)
        return pltpu.make_async_copy(a_s.at[pl.ds(q0, 128), :], o_h.at[pl.ds(q0, 128), pl.ds(0, 512)], sem_out.at[qb])

    emit_attention(qt_s, k_s, vt_s, wo_ref, a_s, oT_a, oT_b, s_a, s_b, m_a, m_b, lambda qb: out_cp(qb).start())
    for qb in range(16):
        out_cp(qb).wait()
    cp_b.wait()


def scratch_shapes():
    V = pltpu.VMEM
    return [
        V((S_, D_), bf16), V((D_, 3 * D_), bf16), V((D_, D_), bf16), V((L_, D_), bf16),
        V((D_, N_), bf16), V((D_, N_), bf16), V((D_, N_), bf16), V((D_, N_), bf16), V((D_, N_), bf16), V((D_, N_), bf16),
        V((D_,), bf16), V((D_,), bf16),
        V(C_A1.shape, bf16), V(C_AK.shape, bf16), V(C_F2.shape, bf16), V(C_AI.shape, bf16),
        V((D_, S_), bf16), V((S_, D_), bf16), V((D_, S_), bf16), V((D_, D_), bf16), V((D_, D_), bf16),
        V((D_, 128), bf16), V((D_, 128), bf16),
        V((GS, 256, 128), f32), V((GS, 256, 128), f32), V((GS, 8, 128), f32), V((GS, 8, 128), f32),
        V((S_, D_), bf16), V((L_, D_), bf16),
        V((D_, 128), f32), V((D_ * UP + 8, 128), f32), V((D_ * UP + 8, 128), f32),
        V((D_ * VP + 8, 128), f32), V((D_ * VP + 8, 128), f32),
        V((NA * FP + 8, 128), f32), V((4 * TR + 8, 128), f32),
        V((32, 128, D_), bf16), V((32, 4, 128, 128), bf16), V((8, 128, 128), bf16), V((32, 4, 128, 128), f32),
        pltpu.SemaphoreType.DMA((24,)), pltpu.SemaphoreType.DMA((17,)),
    ]


@jax.jit
def pallas_concat_heads__sliding_block__ssm_conv_s4__prompt_kernel(
    A_x, A_wqkv, A_wo, B_u, B_A_re, B_A_im, B_B_re, B_B_im, B_C_re, B_C_im, B_log_dt, B_Dskip,
):
    any_spec = pl.BlockSpec(memory_space=pl.ANY)
    out = pl.pallas_call(
        kernel,
        out_shape=jax.ShapeDtypeStruct((S_, 2 * D_), bf16),
        in_specs=[any_spec] * 16,
        out_specs=any_spec,
        scratch_shapes=scratch_shapes(),
        compiler_params=pltpu.CompilerParams(vmem_limit_bytes=112 * 1024 * 1024),
        name="fused",
    )(A_x.reshape(S_, D_), A_wqkv, A_wo, B_u.reshape(L_, D_), B_A_re, B_A_im, B_B_re, B_B_im, B_C_re, B_C_im,
      B_log_dt, B_Dskip, C_A1, C_AK, C_F2, C_AI)
    return out.reshape(1, S_, 2 * D_)
```

```python
import functools
import contextlib

import jax
import jax.numpy as jnp
import numpy as np
from jax import lax
from jax.experimental import pallas as pl
from jax.experimental.pallas import tpu as pltpu

f32, bf16, u32 = jnp.float32, jnp.bfloat16, jnp.uint32
NT = (((1,), (1,)), ((), ()))
NN = (((1,), (0,)), ((), ()))

S_, D_, H_ = 2048, 512, 32
L_, N_ = 2048, 128
NF = 4096
C2 = float(0.25 * np.log2(np.e))
NEG = -1e30
GS = 4
VP, UP, FP = 65, 49, 129
NA = 24
TR = NA * 32


def _scope(n):
    return contextlib.nullcontext()


def _bf16_round(x):
    x = np.ascontiguousarray(x, dtype=np.float32)
    u = x.view(np.uint32).astype(np.uint64)
    r = ((u + 0x7FFF + ((u >> 16) & 1)) & 0xFFFF0000).astype(np.uint32)
    return r.view(np.float32)


LB = _bf16_round(np.arange(L_, dtype=np.float32)).astype(np.int64)
ALPHAS = list(range(8)) + [256 * m for m in range(1, 9)] + [258, 260, 262, 516, 772]
AIDX = {a: i for i, a in enumerate(ALPHAS)}


def _t_row(t):
    if t < 256:
        return AIDX[t % 8] * 32 + t // 8
    blk = t // 256
    rem = t - 256 * blk
    return AIDX[256 * blk + rem % 8] * 32 + rem // 8


def _pack_rows(x):
    b = _bf16_round(np.asarray(x, dtype=np.float32)).view(np.uint32) >> 16
    return np.ascontiguousarray(b[..., 0::2, :] | (b[..., 1::2, :] << 16)).astype(np.uint32)


def _build_consts():
    k1 = np.arange(8)
    A1 = np.zeros((16, 256, 128))
    for g in range(16):
        for n1 in range(8):
            for r in range(16):
                th = 2 * np.pi * (k1 + 0.5) * (256 * n1 + 16 * g + r) / NF
                A1[g, k1 * 32 + r, n1 * 16 + r] = np.cos(th)
                A1[g, k1 * 32 + 16 + r, n1 * 16 + r] = -np.sin(th)
    n2 = np.arange(64)
    k2 = np.arange(64)
    F2 = np.zeros((12, 128, 128))
    perm = np.array([8 * r + a for a in range(8) for r in range(8)])
    for q in range(4):
        ang = -2 * np.pi * (k2[:, None] * n2[None, :] / 64 + q * n2[None, :] / 256)
        Fr, Fi = np.cos(ang), np.sin(ang)
        F2[q] = np.block([[Fr, -Fi], [Fi, Fr]])
        F2[4 + q] = np.block([[Fr[:, perm], -Fi[:, perm]], [Fi[:, perm], Fr[:, perm]]])
        Gr, Gi = Fr.T, -Fi.T
        rp = np.array([16 * g + 2 * s_ + h for g in range(4) for h in range(2) for s_ in range(8)])
        F2[8 + q] = np.block([[Gr[rp], -Gi[rp]], [Gi[rp], Gr[rp]]])
    p16 = np.array([16 * (j // 16) + (j % 16) // 2 + 8 * (j % 2) for j in range(128)])
    F2 = F2[:, :, p16]
    AK = np.zeros((32, 128, 128))
    tiles = []
    for i in range(4):
        for a in range(8):
            starts = []
            for blk in range(8):
                rows = [_t_row(int(LB[256 * blk + 8 * (8 * i + r) + a])) for r in range(8)]
                todo = set(range(8))
                while todo:
                    r0 = min(todo)
                    if all(rows[r] == rows[r0] - r0 + r for r in todo):
                        st = rows[r0] - r0
                    else:
                        st = min(rows[r] for r in todo)
                    v = len(starts)
                    starts.append(st)
                    for r in sorted(todo):
                        if st <= rows[r] < st + 8:
                            th = 2 * np.pi * (k1 + 0.5) * (256 * blk + 8 * (8 * i + r) + a) / NF
                            AK[i * 8 + a, k1 * 16 + r, v * 8 + rows[r] - st] += np.cos(th)
                            AK[i * 8 + a, k1 * 16 + 8 + r, v * 8 + rows[r] - st] += -np.sin(th)
                            todo.discard(r)
            tiles.append(starts)
    AI = np.zeros((32, 64, 128))
    for g8 in range(32):
        for n1 in range(8):
            for r in range(8):
                th = 2 * np.pi * (k1 + 0.5) * (256 * n1 + 16 * (g8 // 2) + 2 * r + (g8 % 2)) / NF
                AI[g8, n1 * 8 + r, k1 * 16 + r] = np.cos(th) * (2.0 / NF)
                AI[g8, n1 * 8 + r, k1 * 16 + 8 + r] = -np.sin(th) * (2.0 / NF)
    return _pack_rows(A1), _pack_rows(AK), _pack_rows(F2), _pack_rows(AI), tiles


C_A1, C_AK, C_F2, C_AI, KT = _build_consts()
L_HI = float(np.array([0x3FB8AA00], dtype=np.uint32).view(np.float32)[0])
L_LO = float(1.4426950408889634 - L_HI)


def loop(lo, hi, body, name):
    if name in "kg,f1u,f1k,i1".split(","):
        for i in range(lo, hi):
            body(i, 0)
    else:
        lax.fori_loop(lo, hi, body, 0)


def al(x, m):
    return x if isinstance(x, int) else pl.multiple_of(x, m)


def ld16(w):
    return pltpu.bitcast(w, bf16)


def q16(x):
    return pltpu.bitcast(x.astype(bf16), u32)


def pck(a, b):
    return pltpu.pack_elementwise([a, b], packed_dtype=bf16)


def unp(w, i):
    return pltpu.unpack_elementwise(w, index=i, packed_dtype=bf16, unpacked_dtype=f32)


def pk16(x):
    ws = [pltpu.pack_elementwise([x[16 * i:16 * i + 8], x[16 * i + 8:16 * i + 16]], packed_dtype=bf16)
          for i in range(x.shape[0] // 16)]
    return ws[0] if len(ws) == 1 else jnp.concatenate(ws, axis=0)


def cmul(a, b):
    return (a[0] * b[0] - a[1] * b[1], a[0] * b[1] + a[1] * b[0])


def csq(a):
    return ((a[0] - a[1]) * (a[0] + a[1]), 2.0 * a[0] * a[1])


def sincos(x):
    kf = jnp.floor(x * 0.6366197723675814 + 0.5)
    r = ((x - kf * 1.5703125) - kf * 4.837512969970703125e-4) - kf * 7.54978995489188216e-8
    z = r * r
    s = ((-1.9515295891e-4 * z + 8.3321608736e-3) * z - 1.6666654611e-1) * z * r + r
    c = ((2.443315711809948e-5 * z - 1.388731625493765e-3) * z + 4.166664568298827e-2) * z * z - 0.5 * z + 1.0
    k = kf.astype(jnp.int32)
    swap = (k & 1) == 1
    s2 = jnp.where(swap, c, s)
    c2 = jnp.where(swap, s, c)
    s3 = jnp.where((k & 2) == 2, -s2, s2)
    c3 = jnp.where(((k + 1) & 2) == 2, -c2, c2)
    return s3, c3


def cexp(a, ph):
    e = jnp.exp(a)
    s, c = sincos(ph)
    return (e * c, e * s)


def fwd4(z):
    a0 = (z[0][0] + z[2][0], z[0][1] + z[2][1])
    a1 = (z[0][0] - z[2][0], z[0][1] - z[2][1])
    b0 = (z[1][0] + z[3][0], z[1][1] + z[3][1])
    b1 = (z[1][0] - z[3][0], z[1][1] - z[3][1])
    return [(a0[0] + b0[0], a0[1] + b0[1]), (a1[0] + b1[1], a1[1] - b1[0]),
            (a0[0] - b0[0], a0[1] - b0[1]), (a1[0] - b1[1], a1[1] + b1[0])]


def inv4(w):
    a0 = (w[0][0] + w[2][0], w[0][1] + w[2][1])
    a1 = (w[0][0] - w[2][0], w[0][1] - w[2][1])
    b0 = (w[1][0] + w[3][0], w[1][1] + w[3][1])
    b1 = (w[1][0] - w[3][0], w[1][1] - w[3][1])
    return [(a0[0] + b0[0], a0[1] + b0[1]), (a1[0] - b1[1], a1[1] + b1[0]),
            (a0[0] - b0[0], a0[1] - b0[1]), (a1[0] + b1[1], a1[1] - b1[0])]


def emit_dt(ldt_ref, dt_s):
    x = ldt_ref[...].astype(f32).reshape(1, D_)
    e = jnp.exp2(x * L_HI)
    e = e + e * ((x * L_LO) * 0.6931471805599453)
    dt = e.astype(bf16).astype(f32)
    for c in range(4):
        dt_s[c * 128:(c + 1) * 128, :] = jnp.broadcast_to(dt[:, c * 128:(c + 1) * 128], (128, 128)).T


def pack2(a, b):
    return pltpu.pack_elementwise([a, b], packed_dtype=bf16)


def emit_pow(r0, RB, prm, dt_s, Ut, Vt, dep=None):
    are_ref, aim_ref, bre_ref, bim_ref, cre_ref, cim_ref = prm
    sl = pl.ds(r0, RB)
    c = r0 // 128
    g0 = r0 % 128
    vbase = g0 * VP + c * 16
    ubase = g0 * UP + c * 12
    dtb = dt_s[sl, :]
    if dep is not None:
        dtb = jnp.where(dep[0], dep[1], dtb)
    a = dtb * are_ref[sl, :].astype(f32)
    ph = dtb * aim_ref[sl, :].astype(f32)
    w = cmul((cre_ref[sl, :].astype(f32), cim_ref[sl, :].astype(f32)),
             (dtb * bre_ref[sl, :].astype(f32), dtb * bim_ref[sl, :].astype(f32)))
    l1 = cexp(a, ph)
    l256 = cexp(a * 256.0, ph * 256.0)
    l2 = csq(l1)
    l4 = csq(l2)
    l8 = csq(l4)
    v1 = (l8[0], -l8[1])
    if 2 == 2:
        v2 = csq(v1)
        ve, vo = (jnp.ones_like(a), jnp.zeros_like(a)), v1
        for j in range(16):
            for ri in range(2):
                Vt[ri][pl.ds(vbase + j, RB, stride=VP), :] = pack2(ve[ri], vo[ri])
            if j < 15:
                ve = v2 if j == 0 else cmul(ve, v2)
                vo = cmul(vo, v2)
    else:
        ve, vo = (jnp.ones_like(a), jnp.zeros_like(a)), v1
        for j in range(16):
            for ri in range(2):
                Vt[ri][pl.ds(vbase + j, RB, stride=VP), :] = pack2(ve[ri], vo[ri])
            if j < 15:
                ve = cmul(vo, v1)
                vo = cmul(ve, v1)
    if dep is not None and 1:
        w = (jnp.where(dep[0], vo[0], w[0]), jnp.where(dep[0], vo[0], w[1]))
    U = {0: w}
    for a_ in range(1, 8):
        U[a_] = cmul(U[a_ - 1], l1)
    for m in range(1, 9):
        U[256 * m] = cmul(U[256 * (m - 1)], l256)
    U[258] = cmul(U[256], l2)
    U[260] = cmul(U[256], l4)
    U[262] = cmul(U[260], l2)
    U[516] = cmul(U[512], l4)
    U[772] = cmul(U[768], l4)
    lst = [U[a_] for a_ in ALPHAS]
    lst = lst + [lst[-1]] * (24 - len(lst))
    for j in range(12):
        for ri in range(2):
            Ut[ri][pl.ds(ubase + j, RB, stride=UP), :] = pack2(lst[2 * j][ri], lst[2 * j + 1][ri])
    return (U[772][0] if 1 else vo[0])


def emit_kgen(g, Ut, Vt, Fs):
    lane = lax.broadcasted_iota(jnp.int32, (24, 128), 1)
    Lm = jnp.concatenate([pltpu.bitcast(Ut[ri][pl.ds(g * UP, 48), :], bf16) for ri in range(2)], axis=1)
    Rm = jnp.concatenate([pltpu.bitcast(Vt[ri][pl.ds(g * VP, 64), :], bf16) for ri in range(2)], axis=1)
    out = lax.dot_general(Lm, Rm, NT, preferred_element_type=f32)
    F = jnp.where(lane < 64, jnp.where(lane < 32, out[0:24], out[24:48]),
                  jnp.where(lane < 96, out[48:72], out[72:96]))
    Fs[pl.ds(g, 24, stride=FP), :] = F


def emit_ttrans(idx, Fs, Ts):
    At = Fs[pl.ds(idx * FP, 128), :].T
    for c in range(4):
        Ts[pl.ds(al(c * TR + idx * 32, 8), 32), :] = At[32 * c:32 * c + 32]


def emit_f1u(gq, c, u_ref, A1_ref, Yu):
    ls = pl.ds(128 * c, 128)
    zs = []
    for j in range(4):
        g = gq + 4 * j
        tile = jnp.concatenate([u_ref[pl.ds(al(256 * n1 + 16 * g, 16), 16), ls] for n1 in range(8)], axis=0)
        zs.append(jnp.dot(ld16(A1_ref[g]), tile, preferred_element_type=f32))
    for k1 in range(8):
        y = fwd4([(zs[j][32 * k1:32 * k1 + 16], zs[j][32 * k1 + 16:32 * k1 + 32]) for j in range(4)])
        for q in range(4):
            for ri in range(2):
                Yu[q * 8 + k1, pl.ds(al(ri * 32 + 8 * gq, 8), 8), ls] = pk16(y[q][ri])


def emit_f1k(a2, c, Ts, AK_ref, Yk):
    zs = [[None, None] for _ in range(4)]
    for aa in range(2):
        a = 2 * a2 + aa
        for i in range(4):
            st = KT[i * 8 + a]
            tile = jnp.concatenate([Ts[pl.ds(c * TR + s0, 8), :] for s0 in st], axis=0)
            zs[i][aa] = jnp.dot(ld16(AK_ref[i * 8 + a])[:, 0:8 * len(st)], tile, preferred_element_type=f32)
    for k1 in range(8):
        zz = []
        for i in range(4):
            re = jnp.concatenate([zs[i][aa][16 * k1:16 * k1 + 8] for aa in range(2)], axis=0)
            im = jnp.concatenate([zs[i][aa][16 * k1 + 8:16 * k1 + 16] for aa in range(2)], axis=0)
            zz.append((re, im))
        y = fwd4(zz)
        for q in range(4):
            for ri in range(2):
                Yk[q * 8 + k1, c, pl.ds(ri * 32 + 8 * a2, 8), :] = pk16(y[q][ri])


def emit_f2(k1s, Yu, Yk, F2_ref, Pb, Zs):
    LAG = 6
    R = Pb.shape[0]
    items = [(k1, c, q) for k1 in k1s for c in range(4) for q in (0, 2, 1, 3)]

    def X(i):
        k1, c, q = items[i]
        Uh = jnp.dot(ld16(F2_ref[q]), ld16(Yu[q * 8 + k1, :, pl.ds(128 * c, 128)]), preferred_element_type=f32)
        Kh = jnp.dot(ld16(F2_ref[4 + q]), ld16(Yk[q * 8 + k1, c]), preferred_element_type=f32)
        Pr = Uh[0:64] * Kh[0:64] - Uh[64:128] * Kh[64:128]
        Pi = Uh[0:64] * Kh[64:128] + Uh[64:128] * Kh[0:64]
        Pb[i % R] = pk16(jnp.concatenate([Pr, Pi], axis=0))

    ws = {}

    def Y(i):
        k1, c, q = items[i]
        W = jnp.dot(ld16(F2_ref[8 + q]), ld16(Pb[i % R]), preferred_element_type=f32)
        ws[q] = (W[0:64], W[64:128])
        if q == 3:
            z = inv4([ws[0], ws[1], ws[2], ws[3]])
            for j in range(4):
                for ri in range(2):
                    for b8 in range(8):
                        Zs[8 * j + b8, c, pl.ds(al(k1 * 16 + ri * 8, 8), 8), :] = z[j][ri][8 * b8:8 * b8 + 8]

    n = len(items)
    for i in range(min(LAG, n)):
        X(i)
    for i in range(n):
        if i + LAG < n:
            X(i + LAG)
        Y(i)


def emit_i1(g16, c, u_ref, dsk, AI_ref, Zs, b_s):
    ls = pl.ds(128 * c, 128)
    ys = [lax.dot_general(ld16(AI_ref[2 * g16 + h]), Zs[2 * g16 + h, c], NN, preferred_element_type=f32) for h in range(2)]
    dk = dsk[:, 128 * c:128 * c + 128]
    for n1 in range(8):
        rows = pl.ds(al(256 * n1 + 16 * g16, 16), 16)
        uw = pltpu.bitcast(u_ref[rows, ls], u32)
        ue, uo = unp(uw, 0), unp(uw, 1)
        yw = pck(ys[0][8 * n1:8 * n1 + 8], ys[1][8 * n1:8 * n1 + 8])
        sw = pck(ue * dk, uo * dk)
        ow = pck(unp(yw, 0) + unp(sw, 0), unp(yw, 1) + unp(sw, 1))
        b_s[rows, ls] = ld16(ow)


def emit_proj(r0, TB, x_ref, wqkv_ref, wqT, wvT, qt_s, k_s, vt_s):
    xb = x_ref[pl.ds(r0, TB), :]
    k_s[pl.ds(al(r0 // 2, TB // 2), TB // 2), :] = q16(jnp.dot(xb, wqkv_ref[:, 512:1024], preferred_element_type=f32))
    qt_s[:, pl.ds(r0, TB)] = q16(lax.dot_general(ld16(wqT[...]), xb, NT, preferred_element_type=f32))
    vt_s[:, pl.ds(r0, TB)] = q16(lax.dot_general(ld16(wvT[...]), xb, NT, preferred_element_type=f32))


def emit_attention(qt_s, k_s, vt_s, wo_p, a_s, oT_a, oT_b, on_s, s_a, s_b, m_a, m_b, after_outproj):
    row = lax.broadcasted_iota(jnp.int32, (64, 128), 0)
    lane64 = lax.broadcasted_iota(jnp.int32, (64, 128), 1) & 63
    near_ok = row <= lane64
    lo8 = lax.broadcasted_iota(jnp.int32, (8, 128), 1) < 64
    lo16 = lax.broadcasted_iota(jnp.int32, (16, 128), 1) < 64
    z8 = jnp.zeros((8, 128), u32)
    z64 = jnp.zeros((64, 128), f32)
    ND = 4
    oTs = (oT_a, oT_b)

    def qk_group(j, par, nch, hg, s_ref, m_ref):
        t0 = al(j * 128, 128)
        wn = al(j * 64 + par * 32, 32)
        ls = pl.ds(hg * 128, 128)
        nmid = min(nch - 1, 3)
        if nch == 5:
            pcs = []
            for i in range(4):
                pcs.append(k_s[pl.ds(al(wn - 128 + 8 * i, 8), 8), ls])
                pcs.append(k_s[pl.ds(al(wn + 8 * i, 8), 8), ls])
            pcs.append(k_s[pl.ds(al(wn - 96, 32), 96), ls])
            Kw = ld16(jnp.concatenate(pcs, axis=0))
        else:
            Kw = ld16(k_s[pl.ds(al(wn - 32 * nmid, 32), 32 * nch), ls])
        for u in range(4):
            p = hg * 4 + u
            qa = qt_s[pl.ds(p * 16, 8), pl.ds(t0, 128)]
            qb = qt_s[pl.ds(p * 16 + 8, 8), pl.ds(t0, 128)]
            if par == 0:
                qb = pltpu.roll(qb, 64, 1)
            else:
                qa = pltpu.roll(qa, 64, 1)
            qa = jnp.where(lo8, qa, z8)
            qb = jnp.where(lo8, z8, qb)
            W = ld16(jnp.concatenate([z8] * (2 * u) + [qa, qb] + [z8] * (6 - 2 * u), axis=0))
            ST = lax.dot_general(Kw, W, NN, preferred_element_type=f32)
            if nch == 5:
                mrg = jnp.concatenate(
                    [jnp.where(near_ok[16 * i:16 * i + 16], ST[32 * i + 16:32 * i + 32], ST[32 * i:32 * i + 16])
                     for i in range(4)], axis=0)
                mid = ST[128:320]
            else:
                mrg = jnp.where(near_ok, ST[64 * nmid:64 * nmid + 64], NEG)
                mid = ST[0:64 * nmid] if nmid else None
            s_ref[u, 0:64] = mrg
            mx = mrg
            if mid is not None:
                s_ref[u, 64:64 + 64 * nmid] = mid
                for i in range(nmid):
                    mx = jnp.maximum(mx, mid[64 * i:64 * i + 64])
            m_ref[u] = jnp.broadcast_to(jnp.max(mx, axis=0, keepdims=True), (8, 128))

    def pv_group(j, par, nch, hg, s_ref, m_ref):
        nmid = min(nch - 1, 3)
        oT_s = oTs[par]
        for u in range(4):
            p = hg * 4 + u
            m8 = m_ref[u]
            dacc = [None] * ND

            def probs(r0, n):
                x = jnp.exp2((s_ref[u, r0:r0 + n] - jnp.concatenate([m8] * (n // 8), axis=0)) * C2)
                for i in range(n // 8):
                    k = (r0 // 8 + i) % ND
                    dacc[k] = x[8 * i:8 * i + 8] if dacc[k] is None else dacc[k] + x[8 * i:8 * i + 8]
                return x

            def vt(tile, n=128):
                return ld16(vt_s[pl.ds(p * 16, 16), pl.ds(al((j + tile) * 128, 128), n)])

            def pv(v, w):
                return lax.dot_general(v, w, NN, preferred_element_type=f32)

            pm = probs(0, 64)
            pd = probs(64, 64 * nmid) if nmid else None
            if nch == 5:
                pf = jnp.where(near_ok, 0.0, pm)
                pn = jnp.where(near_ok, pm, 0.0)
                if par == 0:
                    OT = (pv(vt(0, 64), pn) + pv(vt(-2), jnp.concatenate([pf, pd[0:64]], axis=0))
                          + pv(vt(-1), pd[64:192]))
                else:
                    OT = (pv(vt(-2), jnp.concatenate([z64, pf], axis=0)) + pv(vt(-1), pd[0:128])
                          + pv(vt(0), jnp.concatenate([pd[128:192], pn], axis=0)))
            elif nch == 4:
                OT = pv(vt(-1), pd[0:128]) + pv(vt(0), jnp.concatenate([pd[128:192], pm], axis=0))
            elif nch == 3:
                OT = pv(vt(0, 64), pm) + pv(vt(-1), pd[0:128])
            elif nch == 2:
                OT = pv(vt(0), jnp.concatenate([pd[0:64], pm], axis=0))
            else:
                OT = pv(vt(0, 64), pm)
            dl = [x for x in dacc if x is not None]
            while len(dl) > 1:
                dl = [dl[2 * i] + dl[2 * i + 1] for i in range(len(dl) // 2)] + dl[len(dl) // 2 * 2:]
            den = jnp.sum(dl[0], axis=0, keepdims=True)
            o = jnp.where(lo16, OT[0:16], OT[16:32]) * (1.0 / den)
            oT_s[pl.ds(p * 8, 8), :] = pk16(o)

    def otrans(par):
        Tw = pltpu.bitcast(ld16(oTs[par][...]).T, u32)
        on_s[pl.ds(par * 32, 32), pl.ds(0, 256)] = Tw[0:32]
        on_s[pl.ds(par * 32, 32), pl.ds(256, 256)] = Tw[32:64]

    def outproj(j):
        a_s[pl.ds(al(j * 128, 128), 128), :] = jnp.dot(
            ld16(on_s[...]), ld16(wo_p[...]), preferred_element_type=f32).astype(bf16)
        after_outproj(j)

    bufs = [(s_a, m_a), (s_b, m_b)]
    OPG = 2

    def tile_block(j, nchs, nch_next, j_next, has_prev):
        for t in range(8):
            par, hg = t // 4, t % 4
            if t + 1 < 8:
                qk_group(j, (t + 1) // 4, nchs[(t + 1) // 4], (t + 1) % 4, *bufs[(t + 1) % 2])
            else:
                qk_group(j_next, 0, nch_next, 0, *bufs[0])
            pv_group(j, par, nchs[par], hg, *bufs[t % 2])
            if t == 0 and has_prev:
                otrans(1)
            if t == OPG and has_prev:
                outproj(j - 1)
            if t == 4:
                otrans(0)

    with _scope("s8_peel"):
        qk_group(0, 0, 1, 0, *bufs[0])
        tile_block(0, (1, 2), 3, 1, False)
        tile_block(1, (3, 4), 5, 2, True)

    AU = 2

    def body(it, c):
        for t in range(AU):
            j = 2 + it * AU + t
            jn = j + 1 if t + 1 < AU else (min(j + 1, 15) if isinstance(j, int) else jnp.minimum(j + 1, 15))
            tile_block(j, (5, 5), 5, jn, True)
        return c

    with _scope("s9_attnloop"):
        loop(0, 14 // AU, body, "att")
    with _scope("s9b_lastout"):
        otrans(1)
        outproj(15)


def kernel(x_h, wqkv_h, wo_h, u_h, are_h, aim_h, bre_h, bim_h, cre_h, cim_h, ldt_h, dsk_h,
           A1_h, AK_h, F2_h, AI_h,
           o_h,
           x_ref, wqkv_ref, wo_ref, u_ref, are, aim, bre, bim, cre, cim, ldt_ref, dsk_ref,
           A1_ref, AK_ref, F2_ref, AI_ref,
           qt_s, k_s, vt_s, wqT, wvT, wo_p, oT_a, oT_b, on_s, s_a, s_b, m_a, m_b, a_s, b_s,
           dt_s, Utr, Uti, Vtr, Vti, Fs, Ts, Yu, Yk, Pb, Zs,
           sem_in, sem_out):
    Ut = (Utr, Uti)
    Vt = (Vtr, Vti)
    prm = (are, aim, bre, bim, cre, cim)
    TB = 256
    NB = S_ // TB
    cps = {}
    nsem = [0]

    def mk(name, src, dst):
        cp = pltpu.make_async_copy(src, dst, sem_in.at[nsem[0]])
        nsem[0] += 1
        cps[name] = cp
        return cp

    XS = 3
    mk("wk", wqkv_h.at[:, pl.ds(512, 512)], wqkv_ref.at[:, pl.ds(512, 512)])
    mk("wq", wqkv_h.at[:, pl.ds(0, 512)], wqkv_ref.at[:, pl.ds(0, 512)])
    mk("wv", wqkv_h.at[:, pl.ds(1024, 512)], wqkv_ref.at[:, pl.ds(1024, 512)])
    for i in range(NB):
        mk("x%d" % i, x_h.at[pl.ds(i * TB, TB), :], x_ref.at[pl.ds(i * TB, TB), :])
    mk("ldt", ldt_h, ldt_ref)
    for i, (s, d) in enumerate(zip((are_h, aim_h, bre_h, bim_h, cre_h, cim_h), prm)):
        mk("p%d" % i, s, d)
    mk("u", u_h, u_ref)
    mk("A1", A1_h, A1_ref)
    mk("AK", AK_h, AK_ref)
    mk("F2", F2_h, F2_ref)
    mk("AI", AI_h, AI_ref)
    mk("dsk", dsk_h, dsk_ref)
    mk("wo", wo_h, wo_ref)

    def start(*names):
        for n in names:
            cps[n].start()

    def kproj(r0):
        k_s[pl.ds(al(r0 // 2, TB // 2), TB // 2), :] = q16(
            jnp.dot(x_ref[pl.ds(r0, TB), :], wqkv_ref[:, 512:1024], preferred_element_type=f32))

    def qvproj(r0):
        xb = x_ref[pl.ds(r0, TB), :]
        qt_s[:, pl.ds(r0, TB)] = q16(lax.dot_general(ld16(wqT[...]), xb, NT, preferred_element_type=f32))
        vt_s[:, pl.ds(r0, TB)] = q16(lax.dot_general(ld16(wvT[...]), xb, NT, preferred_element_type=f32))

    def pow_rows(r0, n):
        RB = 8
        PAR = 1
        never = dt_s[pl.ds(0, RB), :] < -1.0
        last = [dt_s[pl.ds(0, RB), :]] * PAR
        for s in range(n // RB):
            dep = (never, last[s % PAR]) if 1 else None
            last[s % PAR] = emit_pow(al(r0 + s * RB, RB), RB, prm, dt_s, Ut, Vt, dep)


    ST = 0
    def waitn(tag, *names):
        with _scope("w_" + tag):
            for n in names:
                cps[n].wait()

    start(*"wk,x0,x1,wq,x2,wv,x3,ldt,x4,x5,p0,p1,p2,p3,p4,p5,x6,x7".split(","))
    waitn("a", "wk", "x0")
    with _scope("s0a"):
        kproj(0)
    waitn("b", "x1")
    with _scope("s0b"):
        kproj(TB)
    waitn("c", "wq", "x2")
    start("u", "A1")
    with _scope("s0c"):
        kproj(2 * TB)
        wqT[...] = pltpu.bitcast(wqkv_ref[:, 0:512].T, u32)
    waitn("d", "wv", "x3", "ldt")
    start("AK", "F2", "AI", "dsk", "wo")
    with _scope("s0d"):
        kproj(3 * TB)
        wvT[...] = pltpu.bitcast(wqkv_ref[:, 1024:1536].T, u32)
        emit_dt(ldt_ref, dt_s)

    PW1 = 176
    PW2 = (512 - PW1) // 2
    waitn("e", "x4", "x5")
    with _scope("s1a"):
        for i in (0, 1):
            qvproj(i * TB)
            kproj((i + 4) * TB)
    waitn("f", "x6", "x7", "p0", "p1", "p2", "p3", "p4", "p5")
    with _scope("s1b"):
        for i in (2, 3):
            qvproj(i * TB)
            kproj((i + 4) * TB)
        pow_rows(0, PW1)

    def proj_body2(it, c):
        for t in range(2):
            qvproj(al((4 + it * 2 + t) * TB, TB))
        pow_rows(PW1 + it * PW2, PW2)
        return c

    with _scope("s2_proj2"):
        loop(0, 2, proj_body2, "p2")

    GU = 32

    def kgen_body(i, c):
        for gg in range(GU):
            emit_kgen(i * GU + gg, Ut, Vt, Fs)
        return c

    with _scope("s3_kgen"):
        loop(0, 128 // GU, kgen_body, "kg")

    cps["u"].wait()
    cps["A1"].wait()

    def f1u_body(gq, c):
        for cc in range(4):
            emit_f1u(gq, cc, u_ref, A1_ref, Yu)
        for t in range(6):
            emit_ttrans(gq * 6 + t, Fs, Ts)
        return c

    with _scope("s4_f1u"):
        loop(0, 4, f1u_body, "f1u")

    cps["AK"].wait()

    def f1k_body(cc, c):
        for a2 in range(4):
            emit_f1k(a2, cc, Ts, AK_ref, Yk)
        return c

    with _scope("s5_f1k"):
        loop(0, 4, f1k_body, "f1k")

    cps["F2"].wait()
    F2U = 8

    def f2_body(i, c):
        emit_f2([i * F2U + t for t in range(F2U)], Yu, Yk, F2_ref, Pb, Zs)
        return c

    with _scope("s6_f2"):
        loop(0, 8 // F2U, f2_body, "f2")

    cps["AI"].wait()
    cps["dsk"].wait()
    dsk = dsk_ref[...].astype(f32).reshape(1, D_)
    IU = 4

    def i1_body(i, c):
        for t in range(IU):
            for cc in range(4):
                emit_i1(i * IU + t, cc, u_ref, dsk, AI_ref, Zs, b_s)
        return c

    with _scope("s7_i1"):
        loop(0, 16 // IU, i1_body, "i1")
    cp_b = pltpu.make_async_copy(b_s, o_h.at[:, pl.ds(512, 512)], sem_out.at[16])
    cp_b.start()

    cps["wo"].wait()
    for g_ in range(2):
        for p_ in range(16):
            h_ = 2 * p_ + g_
            wo_p[pl.ds((g_ * 16 + p_) * 8, 8), :] = pk16(wo_ref[pl.ds(16 * h_, 16), :].astype(f32))

    def out_cp(qb):
        q0 = al(qb * 128, 128)
        return pltpu.make_async_copy(a_s.at[pl.ds(q0, 128), :], o_h.at[pl.ds(q0, 128), pl.ds(0, 512)], sem_out.at[qb])

    emit_attention(qt_s, k_s, vt_s, wo_p, a_s, oT_a, oT_b, on_s, s_a, s_b, m_a, m_b, lambda qb: out_cp(qb).start())
    with _scope("sA_outwait"):
        for qb in range(16):
            out_cp(qb).wait()
        cp_b.wait()


def scratch_shapes():
    V = pltpu.VMEM
    return [
        V((S_, D_), bf16), V((D_, 3 * D_), bf16), V((D_, D_), bf16), V((L_, D_), bf16),
        V((D_, N_), bf16), V((D_, N_), bf16), V((D_, N_), bf16), V((D_, N_), bf16), V((D_, N_), bf16), V((D_, N_), bf16),
        V((D_,), bf16), V((D_,), bf16),
        V(C_A1.shape, u32), V(C_AK.shape, u32), V(C_F2.shape, u32), V(C_AI.shape, u32),
        V((D_ // 2, S_), u32), V((S_ // 2, D_), u32), V((D_ // 2, S_), u32), V((D_ // 2, D_), u32), V((D_ // 2, D_), u32), V((D_ // 2, D_), u32),
        V((128, 128), u32), V((128, 128), u32), V((64, D_), u32),
        V((GS, 256, 128), f32), V((GS, 256, 128), f32), V((GS, 8, 128), f32), V((GS, 8, 128), f32),
        V((S_, D_), bf16), V((L_, D_), bf16),
        V((D_, 128), f32), V((128 * UP + 8, 128), u32), V((128 * UP + 8, 128), u32),
        V((128 * VP + 8, 128), u32), V((128 * VP + 8, 128), u32),
        V((NA * FP + 8, 128), f32), V((4 * TR + 8, 128), f32),
        V((32, 64, D_), u32), V((32, 4, 64, 128), u32), V((8, 64, 128), u32), V((32, 4, 128, 128), f32),
        pltpu.SemaphoreType.DMA((24,)), pltpu.SemaphoreType.DMA((17,)),
    ]


@jax.jit
def pallas_concat_heads__sliding_block__ssm_conv_s4__prompt_kernel(
    A_x, A_wqkv, A_wo, B_u, B_A_re, B_A_im, B_B_re, B_B_im, B_C_re, B_C_im, B_log_dt, B_Dskip,
):
    any_spec = pl.BlockSpec(memory_space=pl.ANY)
    out = pl.pallas_call(
        kernel,
        out_shape=jax.ShapeDtypeStruct((S_, 2 * D_), bf16),
        in_specs=[any_spec] * 16,
        out_specs=any_spec,
        scratch_shapes=scratch_shapes(),
        compiler_params=pltpu.CompilerParams(vmem_limit_bytes=112 * 1024 * 1024),
        name="fused",
    )(A_x.reshape(S_, D_), A_wqkv, A_wo, B_u.reshape(L_, D_), B_A_re, B_A_im, B_B_re, B_B_im, B_C_re, B_C_im,
      B_log_dt, B_Dskip, C_A1, C_AK, C_F2, C_AI)
    return out.reshape(1, S_, 2 * D_)
```

```python
import functools
import contextlib

import jax
import jax.numpy as jnp
import numpy as np
from jax import lax
from jax.experimental import pallas as pl
from jax.experimental.pallas import tpu as pltpu

f32, bf16, u32 = jnp.float32, jnp.bfloat16, jnp.uint32
NT = (((1,), (1,)), ((), ()))
NN = (((1,), (0,)), ((), ()))

S_, D_, H_ = 2048, 512, 32
L_, N_ = 2048, 128
NF = 4096
C2 = float(0.25 * np.log2(np.e))
NEG = -1e30
GS = 4
VP, UP, FP = 65, 49, 129
NA = 24
TR = NA * 32


def _scope(n):
    return contextlib.nullcontext()


def _bf16_round(x):
    x = np.ascontiguousarray(x, dtype=np.float32)
    u = x.view(np.uint32).astype(np.uint64)
    r = ((u + 0x7FFF + ((u >> 16) & 1)) & 0xFFFF0000).astype(np.uint32)
    return r.view(np.float32)


LB = _bf16_round(np.arange(L_, dtype=np.float32)).astype(np.int64)
ALPHAS = list(range(8)) + [256 * m for m in range(1, 9)] + [258, 260, 262, 516, 772]
AIDX = {a: i for i, a in enumerate(ALPHAS)}


def _t_row(t):
    if t < 256:
        return AIDX[t % 8] * 32 + t // 8
    blk = t // 256
    rem = t - 256 * blk
    return AIDX[256 * blk + rem % 8] * 32 + rem // 8


def _pack_rows(x):
    b = _bf16_round(np.asarray(x, dtype=np.float32)).view(np.uint32) >> 16
    return np.ascontiguousarray(b[..., 0::2, :] | (b[..., 1::2, :] << 16)).astype(np.uint32)


def _build_consts():
    k1 = np.arange(8)
    A1 = np.zeros((16, 256, 128))
    for g in range(16):
        for n1 in range(8):
            for r in range(16):
                th = 2 * np.pi * (k1 + 0.5) * (256 * n1 + 16 * g + r) / NF
                A1[g, k1 * 32 + r, n1 * 16 + r] = np.cos(th)
                A1[g, k1 * 32 + 16 + r, n1 * 16 + r] = -np.sin(th)
    n2 = np.arange(64)
    k2 = np.arange(64)
    F2 = np.zeros((12, 128, 128))
    perm = np.array([8 * r + a for a in range(8) for r in range(8)])
    for q in range(4):
        ang = -2 * np.pi * (k2[:, None] * n2[None, :] / 64 + q * n2[None, :] / 256)
        Fr, Fi = np.cos(ang), np.sin(ang)
        F2[q] = np.block([[Fr, -Fi], [Fi, Fr]])
        F2[4 + q] = np.block([[Fr[:, perm], -Fi[:, perm]], [Fi[:, perm], Fr[:, perm]]])
        Gr, Gi = Fr.T, -Fi.T
        rp = np.array([16 * g + 2 * s_ + h for g in range(4) for h in range(2) for s_ in range(8)])
        F2[8 + q] = np.block([[Gr[rp], -Gi[rp]], [Gi[rp], Gr[rp]]])
    p16 = np.array([16 * (j // 16) + (j % 16) // 2 + 8 * (j % 2) for j in range(128)])
    F2 = F2[:, :, p16]
    AK = np.zeros((32, 128, 128))
    tiles = []
    for i in range(4):
        for a in range(8):
            starts = []
            for blk in range(8):
                rows = [_t_row(int(LB[256 * blk + 8 * (8 * i + r) + a])) for r in range(8)]
                todo = set(range(8))
                while todo:
                    r0 = min(todo)
                    if all(rows[r] == rows[r0] - r0 + r for r in todo):
                        st = rows[r0] - r0
                    else:
                        st = min(rows[r] for r in todo)
                    v = len(starts)
                    starts.append(st)
                    for r in sorted(todo):
                        if st <= rows[r] < st + 8:
                            th = 2 * np.pi * (k1 + 0.5) * (256 * blk + 8 * (8 * i + r) + a) / NF
                            AK[i * 8 + a, k1 * 16 + r, v * 8 + rows[r] - st] += np.cos(th)
                            AK[i * 8 + a, k1 * 16 + 8 + r, v * 8 + rows[r] - st] += -np.sin(th)
                            todo.discard(r)
            tiles.append(starts)
    AI = np.zeros((32, 64, 128))
    for g8 in range(32):
        for n1 in range(8):
            for r in range(8):
                th = 2 * np.pi * (k1 + 0.5) * (256 * n1 + 16 * (g8 // 2) + 2 * r + (g8 % 2)) / NF
                AI[g8, n1 * 8 + r, k1 * 16 + r] = np.cos(th) * (2.0 / NF)
                AI[g8, n1 * 8 + r, k1 * 16 + 8 + r] = -np.sin(th) * (2.0 / NF)
    return _pack_rows(A1), _pack_rows(AK), _pack_rows(F2), _pack_rows(AI), tiles


C_A1, C_AK, C_F2, C_AI, KT = _build_consts()
L_HI = float(np.array([0x3FB8AA00], dtype=np.uint32).view(np.float32)[0])
L_LO = float(1.4426950408889634 - L_HI)


def loop(lo, hi, body, name):
    if name in "kg,f1u,f1k,i1".split(","):
        for i in range(lo, hi):
            body(i, 0)
    else:
        lax.fori_loop(lo, hi, body, 0)


def al(x, m):
    return x if isinstance(x, int) else pl.multiple_of(x, m)


def ld16(w):
    return pltpu.bitcast(w, bf16)


def q16(x):
    return pltpu.bitcast(x.astype(bf16), u32)


def pck(a, b):
    return pltpu.pack_elementwise([a, b], packed_dtype=bf16)


def unp(w, i):
    return pltpu.unpack_elementwise(w, index=i, packed_dtype=bf16, unpacked_dtype=f32)


def pk16(x):
    ws = [pltpu.pack_elementwise([x[16 * i:16 * i + 8], x[16 * i + 8:16 * i + 16]], packed_dtype=bf16)
          for i in range(x.shape[0] // 16)]
    return ws[0] if len(ws) == 1 else jnp.concatenate(ws, axis=0)


def cmul(a, b):
    return (a[0] * b[0] - a[1] * b[1], a[0] * b[1] + a[1] * b[0])


def csq(a):
    return ((a[0] - a[1]) * (a[0] + a[1]), 2.0 * a[0] * a[1])


def sincos(x):
    kf = jnp.floor(x * 0.6366197723675814 + 0.5)
    r = ((x - kf * 1.5703125) - kf * 4.837512969970703125e-4) - kf * 7.54978995489188216e-8
    z = r * r
    s = ((-1.9515295891e-4 * z + 8.3321608736e-3) * z - 1.6666654611e-1) * z * r + r
    c = ((2.443315711809948e-5 * z - 1.388731625493765e-3) * z + 4.166664568298827e-2) * z * z - 0.5 * z + 1.0
    k = kf.astype(jnp.int32)
    swap = (k & 1) == 1
    s2 = jnp.where(swap, c, s)
    c2 = jnp.where(swap, s, c)
    s3 = jnp.where((k & 2) == 2, -s2, s2)
    c3 = jnp.where(((k + 1) & 2) == 2, -c2, c2)
    return s3, c3


def cexp(a, ph):
    e = jnp.exp(a)
    s, c = sincos(ph)
    return (e * c, e * s)


def fwd4(z):
    a0 = (z[0][0] + z[2][0], z[0][1] + z[2][1])
    a1 = (z[0][0] - z[2][0], z[0][1] - z[2][1])
    b0 = (z[1][0] + z[3][0], z[1][1] + z[3][1])
    b1 = (z[1][0] - z[3][0], z[1][1] - z[3][1])
    return [(a0[0] + b0[0], a0[1] + b0[1]), (a1[0] + b1[1], a1[1] - b1[0]),
            (a0[0] - b0[0], a0[1] - b0[1]), (a1[0] - b1[1], a1[1] + b1[0])]


def inv4(w):
    a0 = (w[0][0] + w[2][0], w[0][1] + w[2][1])
    a1 = (w[0][0] - w[2][0], w[0][1] - w[2][1])
    b0 = (w[1][0] + w[3][0], w[1][1] + w[3][1])
    b1 = (w[1][0] - w[3][0], w[1][1] - w[3][1])
    return [(a0[0] + b0[0], a0[1] + b0[1]), (a1[0] - b1[1], a1[1] + b1[0]),
            (a0[0] - b0[0], a0[1] - b0[1]), (a1[0] + b1[1], a1[1] - b1[0])]


def emit_dt(ldt_ref, dt_s):
    x = ldt_ref[...].astype(f32).reshape(1, D_)
    e = jnp.exp2(x * L_HI)
    e = e + e * ((x * L_LO) * 0.6931471805599453)
    dt = e.astype(bf16).astype(f32)
    for c in range(4):
        dt_s[c * 128:(c + 1) * 128, :] = jnp.broadcast_to(dt[:, c * 128:(c + 1) * 128], (128, 128)).T


def pack2(a, b):
    return pltpu.pack_elementwise([a, b], packed_dtype=bf16)


def emit_pow(r0, RB, prm, dt_s, Ut, Vt, dep=None):
    are_ref, aim_ref, bre_ref, bim_ref, cre_ref, cim_ref = prm
    sl = pl.ds(r0, RB)
    c = r0 // 128
    g0 = r0 % 128
    vbase = g0 * VP + c * 16
    ubase = g0 * UP + c * 12
    dtb = dt_s[sl, :]
    if dep is not None:
        dtb = jnp.where(dep[0], dep[1], dtb)
    a = dtb * are_ref[sl, :].astype(f32)
    ph = dtb * aim_ref[sl, :].astype(f32)
    w = cmul((cre_ref[sl, :].astype(f32), cim_ref[sl, :].astype(f32)),
             (dtb * bre_ref[sl, :].astype(f32), dtb * bim_ref[sl, :].astype(f32)))
    l1 = cexp(a, ph)
    l256 = cexp(a * 256.0, ph * 256.0)
    l2 = csq(l1)
    l4 = csq(l2)
    l8 = csq(l4)
    v1 = (l8[0], -l8[1])
    if 2 == 2:
        v2 = csq(v1)
        ve, vo = (jnp.ones_like(a), jnp.zeros_like(a)), v1
        for j in range(16):
            for ri in range(2):
                Vt[ri][pl.ds(vbase + j, RB, stride=VP), :] = pack2(ve[ri], vo[ri])
            if j < 15:
                ve = v2 if j == 0 else cmul(ve, v2)
                vo = cmul(vo, v2)
    else:
        ve, vo = (jnp.ones_like(a), jnp.zeros_like(a)), v1
        for j in range(16):
            for ri in range(2):
                Vt[ri][pl.ds(vbase + j, RB, stride=VP), :] = pack2(ve[ri], vo[ri])
            if j < 15:
                ve = cmul(vo, v1)
                vo = cmul(ve, v1)
    if dep is not None and 1:
        w = (jnp.where(dep[0], vo[0], w[0]), jnp.where(dep[0], vo[0], w[1]))
    def put(j, x, y):
        for ri in range(2):
            Ut[ri][pl.ds(ubase + j, RB, stride=UP), :] = pack2(x[ri], y[ri])

    u0 = w
    for j in range(4):
        u1 = cmul(u0, l1)
        put(j, u0, u1)
        if j < 3:
            u0 = cmul(u1, l1)
    u256 = cmul(w, l256)
    u512 = cmul(u256, l256)
    put(4, u256, u512)
    u260 = cmul(u256, l4)
    put(8, cmul(u256, l2), u260)
    put(9, cmul(u260, l2), cmul(u512, l4))
    ua = cmul(u512, l256)
    u772 = cmul(ua, l4)
    put(10, u772, u772)
    put(11, u772, u772)
    ub = cmul(ua, l256)
    put(5, ua, ub)
    ua = cmul(ub, l256)
    ub = cmul(ua, l256)
    put(6, ua, ub)
    ua = cmul(ub, l256)
    ub = cmul(ua, l256)
    put(7, ua, ub)
    return ub[0]


def emit_kgen(g, Ut, Vt, Fs):
    lane = lax.broadcasted_iota(jnp.int32, (24, 128), 1)
    Lm = jnp.concatenate([pltpu.bitcast(Ut[ri][pl.ds(g * UP, 48), :], bf16) for ri in range(2)], axis=1)
    Rm = jnp.concatenate([pltpu.bitcast(Vt[ri][pl.ds(g * VP, 64), :], bf16) for ri in range(2)], axis=1)
    out = lax.dot_general(Lm, Rm, NT, preferred_element_type=f32)
    F = jnp.where(lane < 64, jnp.where(lane < 32, out[0:24], out[24:48]),
                  jnp.where(lane < 96, out[48:72], out[72:96]))
    Fs[pl.ds(g, 24, stride=FP), :] = F


def emit_ttrans(idx, Fs, Ts):
    At = Fs[pl.ds(idx * FP, 128), :].T
    for c in range(4):
        Ts[pl.ds(al(c * TR + idx * 32, 8), 32), :] = At[32 * c:32 * c + 32]


def emit_f1u(gq, c, u_ref, A1_ref, Yu):
    ls = pl.ds(128 * c, 128)
    zs = []
    for j in range(4):
        g = gq + 4 * j
        tile = jnp.concatenate([u_ref[pl.ds(al(256 * n1 + 16 * g, 16), 16), ls] for n1 in range(8)], axis=0)
        zs.append(jnp.dot(ld16(A1_ref[g]), tile, preferred_element_type=f32))
    for k1 in range(8):
        y = fwd4([(zs[j][32 * k1:32 * k1 + 16], zs[j][32 * k1 + 16:32 * k1 + 32]) for j in range(4)])
        for q in range(4):
            for ri in range(2):
                Yu[q * 8 + k1, pl.ds(al(ri * 32 + 8 * gq, 8), 8), ls] = pk16(y[q][ri])


def emit_f1k(a2, c, Ts, AK_ref, Yk):
    zs = [[None, None] for _ in range(4)]
    for aa in range(2):
        a = 2 * a2 + aa
        for i in range(4):
            st = KT[i * 8 + a]
            tile = jnp.concatenate([Ts[pl.ds(c * TR + s0, 8), :] for s0 in st], axis=0)
            zs[i][aa] = jnp.dot(ld16(AK_ref[i * 8 + a])[:, 0:8 * len(st)], tile, preferred_element_type=f32)
    for k1 in range(8):
        zz = []
        for i in range(4):
            re = jnp.concatenate([zs[i][aa][16 * k1:16 * k1 + 8] for aa in range(2)], axis=0)
            im = jnp.concatenate([zs[i][aa][16 * k1 + 8:16 * k1 + 16] for aa in range(2)], axis=0)
            zz.append((re, im))
        y = fwd4(zz)
        for q in range(4):
            for ri in range(2):
                Yk[q * 8 + k1, c, pl.ds(ri * 32 + 8 * a2, 8), :] = pk16(y[q][ri])


def emit_f2(k1s, Yu, Yk, F2_ref, Pb, Zs):
    LAG = 6
    R = Pb.shape[0]
    items = [(k1, c, q) for k1 in k1s for c in range(4) for q in (0, 2, 1, 3)]

    def X(i):
        k1, c, q = items[i]
        Uh = jnp.dot(ld16(F2_ref[q]), ld16(Yu[q * 8 + k1, :, pl.ds(128 * c, 128)]), preferred_element_type=f32)
        Kh = jnp.dot(ld16(F2_ref[4 + q]), ld16(Yk[q * 8 + k1, c]), preferred_element_type=f32)
        Pr = Uh[0:64] * Kh[0:64] - Uh[64:128] * Kh[64:128]
        Pi = Uh[0:64] * Kh[64:128] + Uh[64:128] * Kh[0:64]
        Pb[i % R] = pk16(jnp.concatenate([Pr, Pi], axis=0))

    ws = {}

    def Y(i):
        k1, c, q = items[i]
        W = jnp.dot(ld16(F2_ref[8 + q]), ld16(Pb[i % R]), preferred_element_type=f32)
        ws[q] = (W[0:64], W[64:128])
        if q == 3:
            z = inv4([ws[0], ws[1], ws[2], ws[3]])
            for j in range(4):
                for ri in range(2):
                    for b8 in range(8):
                        Zs[8 * j + b8, c, pl.ds(al(k1 * 16 + ri * 8, 8), 8), :] = z[j][ri][8 * b8:8 * b8 + 8]

    n = len(items)
    for i in range(min(LAG, n)):
        X(i)
    for i in range(n):
        if i + LAG < n:
            X(i + LAG)
        Y(i)


def emit_i1(g16, c, u_ref, dsk, AI_ref, Zs, b_s):
    ls = pl.ds(128 * c, 128)
    ys = [lax.dot_general(ld16(AI_ref[2 * g16 + h]), Zs[2 * g16 + h, c], NN, preferred_element_type=f32) for h in range(2)]
    dk = dsk[:, 128 * c:128 * c + 128]
    for n1 in range(8):
        rows = pl.ds(al(256 * n1 + 16 * g16, 16), 16)
        uw = pltpu.bitcast(u_ref[rows, ls], u32)
        ow = pck(ys[0][8 * n1:8 * n1 + 8] + unp(uw, 0) * dk, ys[1][8 * n1:8 * n1 + 8] + unp(uw, 1) * dk)
        b_s[rows, ls] = ld16(ow)


def emit_proj(r0, TB, x_ref, wqkv_ref, wqT, wvT, qt_s, k_s, vt_s):
    xb = x_ref[pl.ds(r0, TB), :]
    k_s[pl.ds(al(r0 // 2, TB // 2), TB // 2), :] = q16(jnp.dot(xb, wqkv_ref[:, 512:1024], preferred_element_type=f32))
    qt_s[:, pl.ds(r0, TB)] = q16(lax.dot_general(ld16(wqT[...]), xb, NT, preferred_element_type=f32))
    vt_s[:, pl.ds(r0, TB)] = q16(lax.dot_general(ld16(wvT[...]), xb, NT, preferred_element_type=f32))


def emit_attention(qt_s, k_s, vt_s, wo_p, a_s, oT_a, oT_b, on_s, s_a, s_b, m_a, m_b, after_outproj, filler, after_peel):
    row = lax.broadcasted_iota(jnp.int32, (64, 128), 0)
    lane64 = lax.broadcasted_iota(jnp.int32, (64, 128), 1) & 63
    near_ok = row <= lane64
    lo8 = lax.broadcasted_iota(jnp.int32, (8, 128), 1) < 64
    lo16 = lax.broadcasted_iota(jnp.int32, (16, 128), 1) < 64
    z8 = jnp.zeros((8, 128), u32)
    z64 = jnp.zeros((64, 128), f32)
    ND = 2
    oTs = (oT_a, oT_b)

    def qk_group(j, par, nch, hg, s_ref, m_ref):
        t0 = al(j * 128, 128)
        wn = al(j * 64 + par * 32, 32)
        ls = pl.ds(hg * 128, 128)
        nmid = min(nch - 1, 3)
        if nch == 5:
            pcs = []
            for i in range(4):
                pcs.append(k_s[pl.ds(al(wn - 128 + 8 * i, 8), 8), ls])
                pcs.append(k_s[pl.ds(al(wn + 8 * i, 8), 8), ls])
            pcs.append(k_s[pl.ds(al(wn - 96, 32), 96), ls])
            Kw = ld16(jnp.concatenate(pcs, axis=0))
        else:
            Kw = ld16(k_s[pl.ds(al(wn - 32 * nmid, 32), 32 * nch), ls])
        for u in range(4):
            p = hg * 4 + u
            qq = qt_s[par, pl.ds(p * 16, 16), pl.ds(t0, 128)]
            W = ld16(jnp.concatenate([z8] * (2 * u) + [qq] + [z8] * (6 - 2 * u), axis=0))
            ST = lax.dot_general(Kw, W, NN, preferred_element_type=f32)
            if nch == 5:
                mrg = jnp.concatenate(
                    [jnp.where(near_ok[16 * i:16 * i + 16], ST[32 * i + 16:32 * i + 32], ST[32 * i:32 * i + 16])
                     for i in range(4)], axis=0)
                mid = ST[128:320]
            else:
                mrg = jnp.where(near_ok, ST[64 * nmid:64 * nmid + 64], NEG)
                mid = ST[0:64 * nmid] if nmid else None
            s_ref[u, 0:64] = mrg
            mx = mrg
            if mid is not None:
                s_ref[u, 64:64 + 64 * nmid] = mid
                for i in range(nmid):
                    mx = jnp.maximum(mx, mid[64 * i:64 * i + 64])
            m_ref[u] = jnp.broadcast_to(jnp.max(mx, axis=0, keepdims=True), (8, 128))

    def pv_group(j, par, nch, hg, s_ref, m_ref):
        nmid = min(nch - 1, 3)
        oT_s = oTs[par]
        for u in range(4):
            p = hg * 4 + u
            m8 = m_ref[u]
            dacc = [None] * ND

            def probs(r0, n):
                x = jnp.exp2((s_ref[u, r0:r0 + n] - jnp.concatenate([m8] * (n // 8), axis=0)) * C2)
                for i in range(n // 8):
                    k = (r0 // 8 + i) % ND
                    dacc[k] = x[8 * i:8 * i + 8] if dacc[k] is None else dacc[k] + x[8 * i:8 * i + 8]
                return x

            def vt(tile, n=128):
                return ld16(vt_s[pl.ds(p * 16, 16), pl.ds(al((j + tile) * 128, 128), n)])

            def pv(v, w):
                if 1:
                    w = w.astype(bf16)
                return lax.dot_general(v, w, NN, preferred_element_type=f32)

            pm = probs(0, 64)
            pd = probs(64, 64 * nmid) if nmid else None
            if nch == 5:
                pf = jnp.where(near_ok, 0.0, pm)
                pn = jnp.where(near_ok, pm, 0.0)
                if par == 0:
                    OT = (pv(vt(0, 64), pn) + pv(vt(-2), jnp.concatenate([pf, pd[0:64]], axis=0))
                          + pv(vt(-1), pd[64:192]))
                else:
                    OT = (pv(vt(-2), jnp.concatenate([z64, pf], axis=0)) + pv(vt(-1), pd[0:128])
                          + pv(vt(0), jnp.concatenate([pd[128:192], pn], axis=0)))
            elif nch == 4:
                OT = pv(vt(-1), pd[0:128]) + pv(vt(0), jnp.concatenate([pd[128:192], pm], axis=0))
            elif nch == 3:
                OT = pv(vt(0, 64), pm) + pv(vt(-1), pd[0:128])
            elif nch == 2:
                OT = pv(vt(0), jnp.concatenate([pd[0:64], pm], axis=0))
            else:
                OT = pv(vt(0, 64), pm)
            dl = [x for x in dacc if x is not None]
            while len(dl) > 1:
                dl = [dl[2 * i] + dl[2 * i + 1] for i in range(len(dl) // 2)] + dl[len(dl) // 2 * 2:]
            den = jnp.sum(dl[0], axis=0, keepdims=True)
            o = jnp.where(lo16, OT[0:16], OT[16:32]) * (1.0 / den)
            oT_s[pl.ds(p * 8, 8), :] = pk16(o)

    def otrans(par):
        Tw = pltpu.bitcast(ld16(oTs[par][...]).T, u32)
        on_s[pl.ds(par * 32, 32), pl.ds(0, 256)] = Tw[0:32]
        on_s[pl.ds(par * 32, 32), pl.ds(256, 256)] = Tw[32:64]

    def outproj(j):
        a_s[pl.ds(al(j * 128, 128), 128), :] = jnp.dot(
            ld16(on_s[...]), ld16(wo_p[...]), preferred_element_type=f32).astype(bf16)
        after_outproj(j, None)

    def outproj_half(j, par):
        a_s[pl.ds(j * 128 + par * 64, 64), :] = jnp.dot(
            ld16(on_s[pl.ds(par * 32, 32), :]), ld16(wo_p[...]), preferred_element_type=f32).astype(bf16)
        after_outproj(j, par)

    bufs = [(s_a, m_a), (s_b, m_b)]
    OPG = 2

    def tile_block(j, nchs, nch_next, j_next, has_prev, fill=False):
        for t in range(8):
            par, hg = t // 4, t % 4
            if t + 1 < 8:
                qk_group(j, (t + 1) // 4, nchs[(t + 1) // 4], (t + 1) % 4, *bufs[(t + 1) % 2])
            elif j_next is not None:
                qk_group(j_next, 0, nch_next, 0, *bufs[0])
            pv_group(j, par, nchs[par], hg, *bufs[t % 2])
            if t == 0 and has_prev:
                otrans(1)
            if t == OPG and has_prev:
                outproj(j - 1)
            if t == 4:
                otrans(0)
            if t == 5 and j_next is None:
                outproj_half(j, 0)
            if fill:
                filler(j * 8 + t)

    with _scope("s8_peel"):
        qk_group(0, 0, 1, 0, *bufs[0])
        tile_block(0, (1, 2), 3, 1, False, True)
        tile_block(1, (3, 4), 5, 2, True, True)
    after_peel()

    AU = 2

    def body(it, c):
        for t in range(AU):
            j = 2 + it * AU + t
            tile_block(j, (5, 5), 5, j + 1, True)
        return c

    with _scope("s9_attnloop"):
        loop(0, 6, body, "att")
    with _scope("s9a_last2"):
        tile_block(14, (5, 5), 5, 15, True)
        tile_block(15, (5, 5), None, None, True)
        otrans(1)
        outproj_half(15, 1)


def kernel(x_h, wqkv_h, wo_h, u_h, are_h, aim_h, bre_h, bim_h, cre_h, cim_h, ldt_h, dsk_h,
           A1_h, AK_h, F2_h, AI_h,
           o_h,
           x_ref, wqkv_ref, wo_ref, u_ref, are, aim, bre, bim, cre, cim, ldt_ref, dsk_ref,
           A1_ref, AK_ref, F2_ref, AI_ref,
           qt_s, k_s, vt_s, wqT, wvT, wo_p, oT_a, oT_b, on_s, s_a, s_b, m_a, m_b, a_s, b_s,
           dt_s, Utr, Uti, Vtr, Vti, Fs, Ts, Yu, Yk, Pb, Zs,
           sem_in, sem_out):
    Ut = (Utr, Uti)
    Vt = (Vtr, Vti)
    prm = (are, aim, bre, bim, cre, cim)
    TB = 256
    NB = S_ // TB
    cps = {}
    groups = (("wk", "x0"), ("x1", "x2"), ("wq", "wv", "x3", "ldt"),
              ("x4", "x5", "x6", "x7", "p0", "p1", "p2", "p3", "p4", "p5"),
              ("u", "A1", "AK", "F2", "AI", "dsk", "wo"))
    sem_of = {n: i for i, g in enumerate(groups) for n in g}

    def mk(name, src, dst):
        cps[name] = pltpu.make_async_copy(src, dst, sem_in.at[sem_of[name]])

    mk("wk", wqkv_h.at[:, pl.ds(512, 512)], wqkv_ref.at[:, pl.ds(512, 512)])
    mk("wq", wqkv_h.at[:, pl.ds(0, 512)], wqkv_ref.at[:, pl.ds(0, 512)])
    mk("wv", wqkv_h.at[:, pl.ds(1024, 512)], wqkv_ref.at[:, pl.ds(1024, 512)])
    for i in range(NB):
        mk("x%d" % i, x_h.at[pl.ds(i * TB, TB), :], x_ref.at[pl.ds(i * TB, TB), :])
    mk("ldt", ldt_h, ldt_ref)
    for i, (s, d) in enumerate(zip((are_h, aim_h, bre_h, bim_h, cre_h, cim_h), prm)):
        mk("p%d" % i, s, d)
    mk("u", u_h, u_ref)
    mk("A1", A1_h, A1_ref)
    mk("AK", AK_h, AK_ref)
    mk("F2", F2_h, F2_ref)
    mk("AI", AI_h, AI_ref)
    mk("dsk", dsk_h, dsk_ref)
    mk("wo", wo_h, wo_ref)

    def start(*names):
        for n in names:
            cps[n].start()

    def kproj(r0):
        k_s[pl.ds(al(r0 // 2, TB // 2), TB // 2), :] = q16(
            jnp.dot(x_ref[pl.ds(r0, TB), :], wqkv_ref[:, 512:1024], preferred_element_type=f32))

    def qproj(r0):
        xb = x_ref[pl.ds(r0, TB), :]
        qw = q16(lax.dot_general(ld16(wqT[...]), xb, NT, preferred_element_type=f32))
        lo = lax.broadcasted_iota(jnp.int32, (8, 128), 1) < 64
        z = jnp.zeros((8, 128), u32)
        for c in range(TB // 128):
            nat = qw[:, 128 * c:128 * c + 128]
            rol = pltpu.roll(nat, 64, 1)
            for h in range(H_):
                a_, b_ = nat[8 * h:8 * h + 8], rol[8 * h:8 * h + 8]
                dst = (pl.ds(8 * h, 8), pl.ds(al(r0 + 128 * c, 128), 128))
                if h % 2 == 0:
                    qt_s[(0,) + dst] = jnp.where(lo, a_, z)
                    qt_s[(1,) + dst] = jnp.where(lo, b_, z)
                else:
                    qt_s[(0,) + dst] = jnp.where(lo, z, b_)
                    qt_s[(1,) + dst] = jnp.where(lo, z, a_)

    def vproj(r0):
        xb = x_ref[pl.ds(r0, TB), :]
        vt_s[:, pl.ds(r0, TB)] = q16(lax.dot_general(ld16(wvT[...]), xb, NT, preferred_element_type=f32))

    def qvproj(*r0s):
        for r0 in r0s:
            qproj(r0)
            vproj(r0)

    def pow_rows(r0, n):
        RB = 8
        PAR = 1
        never = dt_s[pl.ds(0, RB), :] < -1.0
        last = [dt_s[pl.ds(0, RB), :]] * PAR
        for s in range(n // RB):
            dep = (never, last[s % PAR]) if 1 else None
            last[s % PAR] = emit_pow(al(r0 + s * RB, RB), RB, prm, dt_s, Ut, Vt, dep)


    ST = 0
    def waitn(tag, *names):
        with _scope("w_" + tag):
            for n in names:
                cps[n].wait()

    start("wk", "x0", "x1", "x2", "wq", "wv", "x3", "ldt", "x4", "x5", "p0", "p1", "p2", "p3", "p4", "p5", "x6", "x7")
    waitn("a", "wk", "x0")
    kproj(0)
    waitn("b", "x1", "x2")
    start("u", "A1")
    kproj(TB)
    kproj(2 * TB)
    waitn("d", "wq", "wv", "x3", "ldt")
    start("AK", "F2", "AI", "dsk", "wo")
    wqT[...] = pltpu.bitcast(wqkv_ref[:, 0:512].T, u32)
    wvT[...] = pltpu.bitcast(wqkv_ref[:, 1024:1536].T, u32)
    kproj(3 * TB)
    emit_dt(ldt_ref, dt_s)
    qvproj(0, TB)

    PW1 = 192
    PW2 = (512 - PW1) // 2
    waitn("f", "x4", "x5", "x6", "x7", "p0", "p1", "p2", "p3", "p4", "p5")
    with _scope("s1b"):
        pow_rows(0, PW1)
        qvproj(2 * TB, 3 * TB)
        for i in (4, 5, 6, 7):
            kproj(i * TB)

    def proj_body2(it, c):
        qvproj(al((4 + it * 2) * TB, TB), al((5 + it * 2) * TB, TB))
        pow_rows(PW1 + it * PW2, PW2)
        return c

    with _scope("s2_proj2"):
        loop(0, 2, proj_body2, "p2")

    waitn("g", "u", "A1", "AK", "F2", "AI", "dsk", "wo")
    GU = 32

    def kgen_body(i, c):
        for gg in range(GU):
            emit_kgen(i * GU + gg, Ut, Vt, Fs)
        return c

    with _scope("s3_kgen"):
        loop(0, 128 // GU, kgen_body, "kg")


    def f1u_body(gq, c):
        for cc in range(4):
            emit_f1u(gq, cc, u_ref, A1_ref, Yu)
        for t in range(6):
            emit_ttrans(gq * 6 + t, Fs, Ts)
        return c

    with _scope("s4_f1u"):
        loop(0, 4, f1u_body, "f1u")


    def f1k_body(cc, c):
        for a2 in range(4):
            emit_f1k(a2, cc, Ts, AK_ref, Yk)
        return c

    with _scope("s5_f1k"):
        loop(0, 4, f1k_body, "f1k")

    F2U = 8

    def f2_body(i, c):
        emit_f2([i * F2U + t for t in range(F2U)], Yu, Yk, F2_ref, Pb, Zs)
        return c

    with _scope("s6_f2"):
        loop(0, 8 // F2U, f2_body, "f2")

    dsk = dsk_ref[...].astype(f32).reshape(1, D_)
    FILL = 1
    cp_b = pltpu.make_async_copy(b_s, o_h.at[:, pl.ds(512, 512)], sem_out)
    if not FILL:
        for g16 in range(16):
            for cc in range(4):
                emit_i1(g16, cc, u_ref, dsk, AI_ref, Zs, b_s)

    def filler(i):
        if FILL:
            for cc in range(4):
                emit_i1(i, cc, u_ref, dsk, AI_ref, Zs, b_s)

    for g_ in range(2):
        for p_ in range(16):
            h_ = 2 * p_ + g_
            wo_p[pl.ds((g_ * 16 + p_) * 8, 8), :] = pk16(wo_ref[pl.ds(16 * h_, 16), :].astype(f32))

    def out_cp(j, half=None):
        if half is None:
            q0, n = al(j * 128, 128), 128
        else:
            q0, n = j * 128 + half * 64, 64
        return pltpu.make_async_copy(a_s.at[pl.ds(q0, n), :], o_h.at[pl.ds(q0, n), pl.ds(0, 512)], sem_out)

    emit_attention(qt_s, k_s, vt_s, wo_p, a_s, oT_a, oT_b, on_s, s_a, s_b, m_a, m_b, lambda j, half: out_cp(j, half).start(), filler, cp_b.start)
    with _scope("sA_outwait"):
        pltpu.make_async_copy(o_h, o_h, sem_out).wait()


def scratch_shapes():
    V = pltpu.VMEM
    return [
        V((S_, D_), bf16), V((D_, 3 * D_), bf16), V((D_, D_), bf16), V((L_, D_), bf16),
        V((D_, N_), bf16), V((D_, N_), bf16), V((D_, N_), bf16), V((D_, N_), bf16), V((D_, N_), bf16), V((D_, N_), bf16),
        V((D_,), bf16), V((D_,), bf16),
        V(C_A1.shape, u32), V(C_AK.shape, u32), V(C_F2.shape, u32), V(C_AI.shape, u32),
        V((2, D_ // 2, S_), u32), V((S_ // 2, D_), u32), V((D_ // 2, S_), u32), V((D_ // 2, D_), u32), V((D_ // 2, D_), u32), V((D_ // 2, D_), u32),
        V((128, 128), u32), V((128, 128), u32), V((64, D_), u32),
        V((GS, 256, 128), f32), V((GS, 256, 128), f32), V((GS, 8, 128), f32), V((GS, 8, 128), f32),
        V((S_, D_), bf16), V((L_, D_), bf16),
        V((D_, 128), f32), V((128 * UP + 8, 128), u32), V((128 * UP + 8, 128), u32),
        V((128 * VP + 8, 128), u32), V((128 * VP + 8, 128), u32),
        V((NA * FP + 8, 128), f32), V((4 * TR + 8, 128), f32),
        V((32, 64, D_), u32), V((32, 4, 64, 128), u32), V((8, 64, 128), u32), V((32, 4, 128, 128), f32),
        pltpu.SemaphoreType.DMA((5,)), pltpu.SemaphoreType.DMA(()),
    ]


@jax.jit
def pallas_concat_heads__sliding_block__ssm_conv_s4__prompt_kernel(
    A_x, A_wqkv, A_wo, B_u, B_A_re, B_A_im, B_B_re, B_B_im, B_C_re, B_C_im, B_log_dt, B_Dskip,
):
    any_spec = pl.BlockSpec(memory_space=pl.ANY)
    out = pl.pallas_call(
        kernel,
        out_shape=jax.ShapeDtypeStruct((S_, 2 * D_), bf16),
        in_specs=[any_spec] * 16,
        out_specs=any_spec,
        scratch_shapes=scratch_shapes(),
        compiler_params=pltpu.CompilerParams(vmem_limit_bytes=112 * 1024 * 1024),
        name="fused",
    )(A_x.reshape(S_, D_), A_wqkv, A_wo, B_u.reshape(L_, D_), B_A_re, B_A_im, B_B_re, B_B_im, B_C_re, B_C_im,
      B_log_dt, B_Dskip, C_A1, C_AK, C_F2, C_AI)
    return out.reshape(1, S_, 2 * D_)
```

```python
import functools
import contextlib

import jax
import jax.numpy as jnp
import numpy as np
from jax import lax
from jax.experimental import pallas as pl
from jax.experimental.pallas import tpu as pltpu

f32, bf16, u32 = jnp.float32, jnp.bfloat16, jnp.uint32
NT = (((1,), (1,)), ((), ()))
NN = (((1,), (0,)), ((), ()))

S_, D_, H_ = 2048, 512, 32
L_, N_ = 2048, 128
NF = 4096
C2 = float(0.25 * np.log2(np.e))
NEG = -1e30
GS = 4
VP, UP, FP = 65, 49, 129
NA = 24
TR = NA * 32
PR = 128 * 17 + 8


def _scope(n):
    return contextlib.nullcontext()


def _bf16_round(x):
    x = np.ascontiguousarray(x, dtype=np.float32)
    u = x.view(np.uint32).astype(np.uint64)
    r = ((u + 0x7FFF + ((u >> 16) & 1)) & 0xFFFF0000).astype(np.uint32)
    return r.view(np.float32)


LB = _bf16_round(np.arange(L_, dtype=np.float32)).astype(np.int64)
ALPHAS = list(range(8)) + [256 * m for m in range(1, 9)] + [258, 260, 262, 516, 772]
AIDX = {a: i for i, a in enumerate(ALPHAS)}


def _t_row(t):
    if t < 256:
        return AIDX[t % 8] * 32 + t // 8
    blk = t // 256
    rem = t - 256 * blk
    return AIDX[256 * blk + rem % 8] * 32 + rem // 8


def _pack_rows(x):
    b = _bf16_round(np.asarray(x, dtype=np.float32)).view(np.uint32) >> 16
    return np.ascontiguousarray(b[..., 0::2, :] | (b[..., 1::2, :] << 16)).astype(np.uint32)


def _build_consts():
    k1 = np.arange(128)
    n1 = np.arange(128)
    A = np.zeros((16, 256, 128))
    AI = np.zeros((16, 128, 256))
    p16 = np.array([16 * (j // 16) + (j % 16) // 2 + 8 * (j % 2) for j in range(256)])
    for n2 in range(16):
        th = 2 * np.pi * (k1[:, None] + 0.5) * (16 * n1[None, :] + n2) / NF
        rows = (k1 // 8) * 16 + k1 % 8
        A[n2, rows] = np.cos(th)
        A[n2, rows + 8] = -np.sin(th)
        AI[n2] = (A[n2].T * (2.0 / NF))[:, p16]
    starts = []
    for n2 in range(16):
        st = []
        for v in range(16):
            rows = [_t_row(int(LB[16 * (8 * v + r) + n2])) for r in range(8)]
            assert all(rows[r] == rows[0] + 2 * r for r in range(8))
            st.append(rows[0])
        starts.append(st)
    return _pack_rows(A), _pack_rows(AI), starts


C_A, C_AI, KST = _build_consts()
L_HI = float(np.array([0x3FB8AA00], dtype=np.uint32).view(np.float32)[0])
L_LO = float(1.4426950408889634 - L_HI)


def loop(lo, hi, body, name):
    if name in "kg,f1u,f1k,i1".split(","):
        for i in range(lo, hi):
            body(i, 0)
    else:
        lax.fori_loop(lo, hi, body, 0)


def al(x, m):
    return x if isinstance(x, int) else pl.multiple_of(x, m)


def ld16(w):
    return pltpu.bitcast(w, bf16)


def q16(x):
    return pltpu.bitcast(x.astype(bf16), u32)


def pck(a, b):
    return pltpu.pack_elementwise([a, b], packed_dtype=bf16)


def unp(w, i):
    return pltpu.unpack_elementwise(w, index=i, packed_dtype=bf16, unpacked_dtype=f32)


def pk16(x):
    ws = [pltpu.pack_elementwise([x[16 * i:16 * i + 8], x[16 * i + 8:16 * i + 16]], packed_dtype=bf16)
          for i in range(x.shape[0] // 16)]
    return ws[0] if len(ws) == 1 else jnp.concatenate(ws, axis=0)


def cmul(a, b):
    return (a[0] * b[0] - a[1] * b[1], a[0] * b[1] + a[1] * b[0])


def csq(a):
    return ((a[0] - a[1]) * (a[0] + a[1]), 2.0 * a[0] * a[1])


def sincos(x):
    kf = jnp.floor(x * 0.6366197723675814 + 0.5)
    r = ((x - kf * 1.5703125) - kf * 4.837512969970703125e-4) - kf * 7.54978995489188216e-8
    z = r * r
    s = ((-1.9515295891e-4 * z + 8.3321608736e-3) * z - 1.6666654611e-1) * z * r + r
    c = ((2.443315711809948e-5 * z - 1.388731625493765e-3) * z + 4.166664568298827e-2) * z * z - 0.5 * z + 1.0
    k = kf.astype(jnp.int32)
    swap = (k & 1) == 1
    s2 = jnp.where(swap, c, s)
    c2 = jnp.where(swap, s, c)
    s3 = jnp.where((k & 2) == 2, -s2, s2)
    c3 = jnp.where(((k + 1) & 2) == 2, -c2, c2)
    return s3, c3


def cexp(a, ph):
    e = jnp.exp(a)
    s, c = sincos(ph)
    return (e * c, e * s)


def fwd4(z):
    a0 = (z[0][0] + z[2][0], z[0][1] + z[2][1])
    a1 = (z[0][0] - z[2][0], z[0][1] - z[2][1])
    b0 = (z[1][0] + z[3][0], z[1][1] + z[3][1])
    b1 = (z[1][0] - z[3][0], z[1][1] - z[3][1])
    return [(a0[0] + b0[0], a0[1] + b0[1]), (a1[0] + b1[1], a1[1] - b1[0]),
            (a0[0] - b0[0], a0[1] - b0[1]), (a1[0] - b1[1], a1[1] + b1[0])]


def inv4(w):
    a0 = (w[0][0] + w[2][0], w[0][1] + w[2][1])
    a1 = (w[0][0] - w[2][0], w[0][1] - w[2][1])
    b0 = (w[1][0] + w[3][0], w[1][1] + w[3][1])
    b1 = (w[1][0] - w[3][0], w[1][1] - w[3][1])
    return [(a0[0] + b0[0], a0[1] + b0[1]), (a1[0] - b1[1], a1[1] + b1[0]),
            (a0[0] - b0[0], a0[1] - b0[1]), (a1[0] + b1[1], a1[1] - b1[0])]


def emit_dt(ldt_ref, dt_s):
    x = ldt_ref[...].astype(f32).reshape(1, D_)
    e = jnp.exp2(x * L_HI)
    e = e + e * ((x * L_LO) * 0.6931471805599453)
    dt = e.astype(bf16).astype(f32)
    for c in range(4):
        dt_s[c * 128:(c + 1) * 128, :] = jnp.broadcast_to(dt[:, c * 128:(c + 1) * 128], (128, 128)).T


def pack2(a, b):
    return pltpu.pack_elementwise([a, b], packed_dtype=bf16)


def emit_pow(r0, RB, prm, dt_s, Ut, Vt, dep=None):
    are_ref, aim_ref, bre_ref, bim_ref, cre_ref, cim_ref = prm
    sl = pl.ds(r0, RB)
    c = r0 // 128
    g0 = r0 % 128
    vbase = g0 * VP + c * 16
    ubase = g0 * UP + c * 12
    dtb = dt_s[sl, :]
    if dep is not None:
        dtb = jnp.where(dep[0], dep[1], dtb)
    a = dtb * are_ref[sl, :].astype(f32)
    ph = dtb * aim_ref[sl, :].astype(f32)
    w = cmul((cre_ref[sl, :].astype(f32), cim_ref[sl, :].astype(f32)),
             (dtb * bre_ref[sl, :].astype(f32), dtb * bim_ref[sl, :].astype(f32)))
    l1 = cexp(a, ph)
    l256 = cexp(a * 256.0, ph * 256.0)
    l2 = csq(l1)
    l4 = csq(l2)
    l8 = csq(l4)
    v1 = (l8[0], -l8[1])
    if 2 == 2:
        v2 = csq(v1)
        ve, vo = (jnp.ones_like(a), jnp.zeros_like(a)), v1
        for j in range(16):
            for ri in range(2):
                Vt[ri][pl.ds(vbase + j, RB, stride=VP), :] = pack2(ve[ri], vo[ri])
            if j < 15:
                ve = v2 if j == 0 else cmul(ve, v2)
                vo = cmul(vo, v2)
    else:
        ve, vo = (jnp.ones_like(a), jnp.zeros_like(a)), v1
        for j in range(16):
            for ri in range(2):
                Vt[ri][pl.ds(vbase + j, RB, stride=VP), :] = pack2(ve[ri], vo[ri])
            if j < 15:
                ve = cmul(vo, v1)
                vo = cmul(ve, v1)
    if dep is not None and 1:
        w = (jnp.where(dep[0], vo[0], w[0]), jnp.where(dep[0], vo[0], w[1]))
    def put(j, x, y):
        for ri in range(2):
            Ut[ri][pl.ds(ubase + j, RB, stride=UP), :] = pack2(x[ri], y[ri])

    u0 = w
    for j in range(4):
        u1 = cmul(u0, l1)
        put(j, u0, u1)
        if j < 3:
            u0 = cmul(u1, l1)
    u256 = cmul(w, l256)
    u512 = cmul(u256, l256)
    put(4, u256, u512)
    u260 = cmul(u256, l4)
    put(8, cmul(u256, l2), u260)
    put(9, cmul(u260, l2), cmul(u512, l4))
    ua = cmul(u512, l256)
    u772 = cmul(ua, l4)
    put(10, u772, u772)
    put(11, u772, u772)
    ub = cmul(ua, l256)
    put(5, ua, ub)
    ua = cmul(ub, l256)
    ub = cmul(ua, l256)
    put(6, ua, ub)
    ua = cmul(ub, l256)
    ub = cmul(ua, l256)
    put(7, ua, ub)
    return ub[0]


def emit_kgen(g, Ut, Vt, Fs):
    lane = lax.broadcasted_iota(jnp.int32, (24, 128), 1)
    Lm = jnp.concatenate([pltpu.bitcast(Ut[ri][pl.ds(g * UP, 48), :], bf16) for ri in range(2)], axis=1)
    Rm = jnp.concatenate([pltpu.bitcast(Vt[ri][pl.ds(g * VP, 64), :], bf16) for ri in range(2)], axis=1)
    out = lax.dot_general(Lm, Rm, NT, preferred_element_type=f32)
    F = jnp.where(lane < 64, jnp.where(lane < 32, out[0:24], out[24:48]),
                  jnp.where(lane < 96, out[48:72], out[72:96]))
    Fs[pl.ds(g, 24, stride=FP), :] = F


def emit_ttrans(idx, Fs, Ts):
    At = Fs[pl.ds(idx * FP, 128), :].T
    for c in range(4):
        Ts[pl.ds(al(c * TR + idx * 32, 8), 32), :] = At[32 * c:32 * c + 32]


def emit_upad(g, u_ref, pad_s):
    for c in range(4):
        w = pltpu.bitcast(u_ref[pl.ds(16 * g, 16), pl.ds(128 * c, 128)], u32)
        for e in range(2):
            pad_s[pl.ds(c * PR + 17 * g + e, 8, stride=2), :] = unp(w, e)


def zrow(c, cc, b):
    return ((c * 4 + cc) * 4 + b) * 256


def emit_f1(b, c, tile, A_ref, Z, zoff):
    zs = [lax.dot_general(ld16(A_ref[4 * a + b]), tile(4 * a + b), NN, preferred_element_type=f32) for a in range(4)]
    for kv in range(16):
        y = _r4([(z[16 * kv:16 * kv + 8], z[16 * kv + 8:16 * kv + 16]) for z in zs], -1)
        for cc in range(4):
            v = _tw(y[cc], b * cc, -1)
            r = zoff + zrow(c, cc, b) + 16 * kv
            Z[pl.ds(al(r, 8), 8), :] = v[0]
            Z[pl.ds(al(r + 8, 8), 8), :] = v[1]


def emit_f1u(b, c, pad_s, A_ref, Z):
    emit_f1(b, c, lambda n2: pad_s[pl.ds(c * PR + n2, 128, stride=17), :], A_ref, Z, ZU)


def emit_f1k(b, c, Ts, A_ref, Z):
    emit_f1(b, c, lambda n2: jnp.concatenate([Ts[pl.ds(c * TR + s0, 8, stride=2), :] for s0 in KST[n2]], axis=0),
            A_ref, Z, ZK)


def _r4(x, sg):
    a0 = (x[0][0] + x[2][0], x[0][1] + x[2][1])
    a1 = (x[0][0] - x[2][0], x[0][1] - x[2][1])
    b0 = (x[1][0] + x[3][0], x[1][1] + x[3][1])
    b1 = (x[1][0] - x[3][0], x[1][1] - x[3][1])
    p = (a1[0] - b1[1], a1[1] + b1[0])
    m = (a1[0] + b1[1], a1[1] - b1[0])
    return [(a0[0] + b0[0], a0[1] + b0[1]), p if sg > 0 else m, (a0[0] - b0[0], a0[1] - b0[1]), m if sg > 0 else p]


def _tw(x, e, sg):
    e = e % 16
    if e == 0:
        return x
    if e == 4:
        return (-x[1], x[0]) if sg > 0 else (x[1], -x[0])
    if e in (2, 6):
        h = float(np.sqrt(0.5))
        if (e == 2) == (sg > 0):
            if e == 2:
                return ((x[0] - x[1]) * h, (x[0] + x[1]) * h)
            return ((x[1] - x[0]) * h, (x[0] + x[1]) * (-h))
        if e == 2:
            return ((x[0] + x[1]) * h, (x[1] - x[0]) * h)
        return ((x[0] + x[1]) * (-h), (x[0] - x[1]) * h)
    c = float(np.cos(2 * np.pi * e / 16))
    s = float(sg * np.sin(2 * np.pi * e / 16))
    return (x[0] * c - x[1] * s, x[0] * s + x[1] * c)


ZU, ZK, ZW = 0, 16384, 32768


def emit_mid(c, cc, kv, Z, z0=0):
    base = zrow(c, cc, 0) + 16 * kv + z0

    def ld(off):
        return [(Z[pl.ds(al(base + off + b * 256, 8), 8), :], Z[pl.ds(al(base + off + b * 256 + 8, 8), 8), :])
                for b in range(4)]

    kh = _r4(ld(ZK), -1)
    uh = _r4(ld(ZU), -1)
    y = _r4([cmul(p, q) for p, q in zip(uh, kh)], +1)
    for b in range(4):
        Z[pl.ds(al(base + ZU + b * 256, 8), 8), :] = y[b][0]
        Z[pl.ds(al(base + ZU + b * 256 + 8, 8), 8), :] = y[b][1]


def emit_inv_a(b, c, Z, zs, Zs):
    IV = 4
    for i, kv in enumerate([h * 8 + j for j in range(8) for h in range(2)]):
        z0 = zs[(i // IV) % len(zs)]
        x = []
        for cc in range(4):
            r = ZU + zrow(c, cc, b) + 16 * kv + z0
            x.append(_tw((Z[pl.ds(al(r, 8), 8), :], Z[pl.ds(al(r + 8, 8), 8), :]), b * cc, +1))
        y = _r4(x, +1)
        for a in range(4):
            Zs[pl.ds((b * 4 + a) * 128 + 8 * kv, 8), :] = pck(y[a][0], y[a][1])


def emit_inv_b(b, t, AI_ref, Zs, pad_s):
    for a in range(4):
        n2 = 4 * a + b
        y = lax.dot_general(ld16(AI_ref[n2]), ld16(Zs[pl.ds((b * 4 + a) * 128, 128), :]), NN, preferred_element_type=f32)
        pad_s[pl.ds(t * PR + n2, 128, stride=17), :] = y


def emit_epilogue(c, t, u_ref, dsk_s, pad_s, b_s, gs=range(128)):
    ls = pl.ds(al(128 * c, 128), 128)
    dk = dsk_s[:, ls]
    for g in gs:
        uw = pltpu.bitcast(u_ref[pl.ds(16 * g, 16), ls], u32)
        ye = pad_s[pl.ds(t * PR + 17 * g, 8, stride=2), :]
        yo = pad_s[pl.ds(t * PR + 17 * g + 1, 8, stride=2), :]
        b_s[pl.ds(16 * g, 16), ls] = ld16(pck(ye + unp(uw, 0) * dk, yo + unp(uw, 1) * dk))


def emit_proj(r0, TB, x_ref, wqkv_ref, wqT, wvT, qt_s, k_s, vt_s):
    xb = x_ref[pl.ds(r0, TB), :]
    k_s[pl.ds(al(r0 // 2, TB // 2), TB // 2), :] = q16(jnp.dot(xb, wqkv_ref[:, 512:1024], preferred_element_type=f32))
    qt_s[:, pl.ds(r0, TB)] = q16(lax.dot_general(ld16(wqT[...]), xb, NT, preferred_element_type=f32))
    vt_s[:, pl.ds(r0, TB)] = q16(lax.dot_general(ld16(wvT[...]), xb, NT, preferred_element_type=f32))


def emit_attention(qt_s, k_s, vt_s, wo_p, a_s, oT_a, oT_b, on_s, s_a, s_b, m_a, m_b, after_outproj, filler):
    row = lax.broadcasted_iota(jnp.int32, (64, 128), 0)
    lane64 = lax.broadcasted_iota(jnp.int32, (64, 128), 1) & 63
    near_ok = row <= lane64
    lo8 = lax.broadcasted_iota(jnp.int32, (8, 128), 1) < 64
    lo16 = lax.broadcasted_iota(jnp.int32, (16, 128), 1) < 64
    z8 = jnp.zeros((8, 128), u32)
    z64 = jnp.zeros((64, 128), f32)
    ND = 2
    oTs = (oT_a, oT_b)

    def qk_group(j, par, nch, hg, s_ref, m_ref):
        t0 = al(j * 128, 128)
        wn = al(j * 64 + par * 32, 32)
        ls = pl.ds(hg * 128, 128)
        nmid = min(nch - 1, 3)
        if nch == 5:
            pcs = []
            for i in range(4):
                pcs.append(k_s[pl.ds(al(wn - 128 + 8 * i, 8), 8), ls])
                pcs.append(k_s[pl.ds(al(wn + 8 * i, 8), 8), ls])
            pcs.append(k_s[pl.ds(al(wn - 96, 32), 96), ls])
            Kw = ld16(jnp.concatenate(pcs, axis=0))
        else:
            Kw = ld16(k_s[pl.ds(al(wn - 32 * nmid, 32), 32 * nch), ls])
        for u in range(4):
            p = hg * 4 + u
            qq = qt_s[par, pl.ds(p * 16, 16), pl.ds(t0, 128)]
            W = ld16(jnp.concatenate([z8] * (2 * u) + [qq] + [z8] * (6 - 2 * u), axis=0))
            ST = lax.dot_general(Kw, W, NN, preferred_element_type=f32)
            if nch == 5:
                mrg = jnp.concatenate(
                    [jnp.where(near_ok[16 * i:16 * i + 16], ST[32 * i + 16:32 * i + 32], ST[32 * i:32 * i + 16])
                     for i in range(4)], axis=0)
                mid = ST[128:320]
            else:
                mrg = jnp.where(near_ok, ST[64 * nmid:64 * nmid + 64], NEG)
                mid = ST[0:64 * nmid] if nmid else None
            s_ref[u, 0:64] = mrg
            mx = mrg
            if mid is not None:
                s_ref[u, 64:64 + 64 * nmid] = mid
                for i in range(nmid):
                    mx = jnp.maximum(mx, mid[64 * i:64 * i + 64])
            m_ref[u] = jnp.broadcast_to(jnp.max(mx, axis=0, keepdims=True), (8, 128))

    def pv_group(j, par, nch, hg, s_ref, m_ref):
        nmid = min(nch - 1, 3)
        oT_s = oTs[par]
        for u in range(4):
            p = hg * 4 + u
            m8 = m_ref[u]
            dacc = [None] * ND

            def probs(r0, n):
                x = jnp.exp2((s_ref[u, r0:r0 + n] - jnp.concatenate([m8] * (n // 8), axis=0)) * C2)
                for i in range(n // 8):
                    k = (r0 // 8 + i) % ND
                    dacc[k] = x[8 * i:8 * i + 8] if dacc[k] is None else dacc[k] + x[8 * i:8 * i + 8]
                return x

            def vt(tile, n=128):
                return ld16(vt_s[pl.ds(p * 16, 16), pl.ds(al((j + tile) * 128, 128), n)])

            def pv(v, w):
                if 1:
                    w = w.astype(bf16)
                return lax.dot_general(v, w, NN, preferred_element_type=f32)

            pm = probs(0, 64)
            pd = probs(64, 64 * nmid) if nmid else None
            if nch == 5:
                pf = jnp.where(near_ok, 0.0, pm)
                pn = jnp.where(near_ok, pm, 0.0)
                if par == 0:
                    OT = (pv(vt(0, 64), pn) + pv(vt(-2), jnp.concatenate([pf, pd[0:64]], axis=0))
                          + pv(vt(-1), pd[64:192]))
                else:
                    OT = (pv(vt(-2), jnp.concatenate([z64, pf], axis=0)) + pv(vt(-1), pd[0:128])
                          + pv(vt(0), jnp.concatenate([pd[128:192], pn], axis=0)))
            elif nch == 4:
                OT = pv(vt(-1), pd[0:128]) + pv(vt(0), jnp.concatenate([pd[128:192], pm], axis=0))
            elif nch == 3:
                OT = pv(vt(0, 64), pm) + pv(vt(-1), pd[0:128])
            elif nch == 2:
                OT = pv(vt(0), jnp.concatenate([pd[0:64], pm], axis=0))
            else:
                OT = pv(vt(0, 64), pm)
            dl = [x for x in dacc if x is not None]
            while len(dl) > 1:
                dl = [dl[2 * i] + dl[2 * i + 1] for i in range(len(dl) // 2)] + dl[len(dl) // 2 * 2:]
            den = jnp.sum(dl[0], axis=0, keepdims=True)
            o = jnp.where(lo16, OT[0:16], OT[16:32]) * (1.0 / den)
            oT_s[pl.ds(p * 8, 8), :] = pk16(o)

    def otrans(par):
        Tw = pltpu.bitcast(ld16(oTs[par][...]).T, u32)
        on_s[pl.ds(par * 32, 32), pl.ds(0, 256)] = Tw[0:32]
        on_s[pl.ds(par * 32, 32), pl.ds(256, 256)] = Tw[32:64]

    def outproj(j):
        a_s[pl.ds(al(j * 128, 128), 128), :] = jnp.dot(
            ld16(on_s[...]), ld16(wo_p[...]), preferred_element_type=f32).astype(bf16)
        after_outproj(j, None)

    def outproj_half(j, par):
        a_s[pl.ds(j * 128 + par * 64, 64), :] = jnp.dot(
            ld16(on_s[pl.ds(par * 32, 32), :]), ld16(wo_p[...]), preferred_element_type=f32).astype(bf16)
        after_outproj(j, par)

    bufs = [(s_a, m_a), (s_b, m_b)]
    OPG = 2

    def tile_block(j, nchs, nch_next, j_next, has_prev, fill=None):
        for t in range(8):
            par, hg = t // 4, t % 4
            if t + 1 < 8:
                qk_group(j, (t + 1) // 4, nchs[(t + 1) // 4], (t + 1) % 4, *bufs[(t + 1) % 2])
            elif j_next is not None:
                qk_group(j_next, 0, nch_next, 0, *bufs[0])
            pv_group(j, par, nchs[par], hg, *bufs[t % 2])
            if t == 0 and has_prev:
                otrans(1)
            if t == OPG and has_prev:
                outproj(j - 1)
            if t == 4:
                otrans(0)
            if t == 5 and j_next is None:
                outproj_half(j, 0)
            if fill is not None:
                fill(t)

    with _scope("s8_peel"):
        qk_group(0, 0, 1, 0, *bufs[0])
        tile_block(0, (1, 2), 3, 1, False, lambda t: filler(0, t))
        tile_block(1, (3, 4), 5, 2, True)

    AU = 2

    def body(it, c):
        for t in range(AU):
            j = 2 + it * AU + t
            tile_block(j, (5, 5), 5, j + 1, True)
        return c

    with _scope("s9_attnloop"):
        loop(0, 6, body, "att")
    with _scope("s9a_last2"):
        tile_block(14, (5, 5), 5, 15, True)
        tile_block(15, (5, 5), None, None, True)
        otrans(1)
        outproj_half(15, 1)


def kernel(x_h, wqkv_h, wo_h, u_h, are_h, aim_h, bre_h, bim_h, cre_h, cim_h, ldt_h, dsk_h,
           A_h, AI_h,
           o_h,
           x_ref, wqkv_ref, wo_ref, u_ref, are, aim, bre, bim, cre, cim, ldt_ref, dsk_ref,
           A_ref, AI_ref,
           qt_s, k_s, vt_s, wqT, wvT, wo_p, oT_a, oT_b, on_s, s_a, s_b, m_a, m_b, a_s, b_s,
           dt_s, Utr, Uti, Vtr, Vti, Fs, Ts, pad_s, Z, Zs, dsk_s,
           sem_in, sem_out):
    Ut = (Utr, Uti)
    Vt = (Vtr, Vti)
    prm = (are, aim, bre, bim, cre, cim)
    TB = 256
    NB = S_ // TB
    cps = {}
    groups = (("wk", "x0"), ("x1", "x2"), ("wq", "wv", "x3", "ldt"),
              ("x4", "x5", "x6", "x7", "p0", "p1", "p2", "p3", "p4", "p5"),
              ("u", "A", "AI", "dsk", "wo"))
    sem_of = {n: i for i, g in enumerate(groups) for n in g}

    def mk(name, src, dst):
        cps[name] = pltpu.make_async_copy(src, dst, sem_in.at[sem_of[name]])

    mk("wk", wqkv_h.at[:, pl.ds(512, 512)], wqkv_ref.at[:, pl.ds(512, 512)])
    mk("wq", wqkv_h.at[:, pl.ds(0, 512)], wqkv_ref.at[:, pl.ds(0, 512)])
    mk("wv", wqkv_h.at[:, pl.ds(1024, 512)], wqkv_ref.at[:, pl.ds(1024, 512)])
    for i in range(NB):
        mk("x%d" % i, x_h.at[pl.ds(i * TB, TB), :], x_ref.at[pl.ds(i * TB, TB), :])
    mk("ldt", ldt_h, ldt_ref)
    for i, (s, d) in enumerate(zip((are_h, aim_h, bre_h, bim_h, cre_h, cim_h), prm)):
        mk("p%d" % i, s, d)
    mk("u", u_h, u_ref)
    mk("A", A_h, A_ref)
    mk("AI", AI_h, AI_ref)
    mk("dsk", dsk_h, dsk_ref)
    mk("wo", wo_h, wo_ref)

    def start(*names):
        for n in names:
            cps[n].start()

    def kproj(r0):
        k_s[pl.ds(al(r0 // 2, TB // 2), TB // 2), :] = q16(
            jnp.dot(x_ref[pl.ds(r0, TB), :], wqkv_ref[:, 512:1024], preferred_element_type=f32))

    def qproj(r0):
        xb = x_ref[pl.ds(r0, TB), :]
        qw = q16(lax.dot_general(ld16(wqT[...]), xb, NT, preferred_element_type=f32))
        lo = lax.broadcasted_iota(jnp.int32, (8, 128), 1) < 64
        z = jnp.zeros((8, 128), u32)
        for c in range(TB // 128):
            nat = qw[:, 128 * c:128 * c + 128]
            rol = pltpu.roll(nat, 64, 1)
            for h in range(H_):
                a_, b_ = nat[8 * h:8 * h + 8], rol[8 * h:8 * h + 8]
                dst = (pl.ds(8 * h, 8), pl.ds(al(r0 + 128 * c, 128), 128))
                if h % 2 == 0:
                    qt_s[(0,) + dst] = jnp.where(lo, a_, z)
                    qt_s[(1,) + dst] = jnp.where(lo, b_, z)
                else:
                    qt_s[(0,) + dst] = jnp.where(lo, z, b_)
                    qt_s[(1,) + dst] = jnp.where(lo, z, a_)

    def vproj(r0):
        xb = x_ref[pl.ds(r0, TB), :]
        vt_s[:, pl.ds(r0, TB)] = q16(lax.dot_general(ld16(wvT[...]), xb, NT, preferred_element_type=f32))

    def qvproj(*r0s):
        for r0 in r0s:
            qproj(r0)
            vproj(r0)

    pow_state = {}

    def pow_gblock(gb):
        never = dt_s[pl.ds(0, 8), :] < -1.0
        last = pow_state.get("last")
        if last is None:
            last = dt_s[pl.ds(0, 8), :]
        for c in range(4):
            last = emit_pow(128 * c + 8 * gb, 8, prm, dt_s, Ut, Vt, (never, last))
        pow_state["last"] = last

    def waitn(tag, *names):
        with _scope("w_" + tag):
            for n in names:
                cps[n].wait()

    start("wk", "x0", "x1", "x2", "wq", "wv", "x3", "ldt", "x4", "x5", "p0", "p1", "p2", "p3", "p4", "p5", "x6", "x7")
    waitn("a", "wk", "x0")
    kproj(0)
    waitn("b", "x1", "x2")
    start("u", "A")
    kproj(TB)
    kproj(2 * TB)
    waitn("d", "wq", "wv", "x3", "ldt")
    start("AI", "dsk", "wo")
    wqT[...] = pltpu.bitcast(wqkv_ref[:, 0:512].T, u32)
    wvT[...] = pltpu.bitcast(wqkv_ref[:, 1024:1536].T, u32)
    kproj(3 * TB)
    emit_dt(ldt_ref, dt_s)
    qvproj(0, TB)

    PB1 = 12
    waitn("f", "x4", "x5", "x6", "x7", "p0", "p1", "p2", "p3", "p4", "p5")
    with _scope("s1b"):
        for gb in range(PB1):
            pow_gblock(gb)
        qvproj(2 * TB, 3 * TB)
        for i in (4, 5, 6, 7):
            kproj(i * TB)
    pow_state.clear()

    waitn("g", "u", "A", "AI", "dsk", "wo")
    dsk_s[...] = dsk_ref[...].astype(f32).reshape(1, D_)
    PST = 14
    with _scope("s3_kgen"):
        for g in range(128):
            if g % PST == 0 and PB1 + g // PST < 16:
                pow_gblock(PB1 + g // PST)
            emit_kgen(g, Ut, Vt, Fs)
            emit_upad(g, u_ref, pad_s)
    with _scope("s4_f1"):
        for i in range(16):
            emit_f1u(i % 4, i // 4, pad_s, A_ref, Z)
            for idx in range(i * 21 // 12, min(21, (i + 1) * 21 // 12)):
                emit_ttrans(idx, Fs, Ts)
        for c in range(4):
            for b in range(4):
                emit_f1k(b, c, Ts, A_ref, Z)

    def b_cp(c):
        l0 = al(128 * c, 128)
        return pltpu.make_async_copy(b_s.at[:, pl.ds(l0, 128)], o_h.at[:, pl.ds(al(512 + l0, 128), 128)], sem_out)

    def zeros_chain(c):
        return [0] if isinstance(c, int) else [((c * (2 * i + 3)) >> 12) * 8 for i in range(3)]

    def mid_c(c):
        zs = zeros_chain(c)
        for i in range(64):
            emit_mid(c, i // 16, i % 16, Z, zs[i % len(zs)])

    def proj_body3(it, c):
        qvproj(al((4 + it) * TB, TB))
        mid_c(it)
        return c

    with _scope("s5_proj3"):
        loop(0, 4, proj_body3, "p3")

    def inv_body(it, carry):
        @pl.when(it > 0)
        def _():
            b_cp(0).start()

        zs = zeros_chain(it)
        for t in range(2):
            c = 2 * it + t
            for b in range(4):
                emit_epilogue(jnp.maximum(c - 1, 0), 1 - t, u_ref, dsk_s, pad_s, b_s, range(32 * b, 32 * b + 32))
                emit_inv_a(b, c, Z, zs, Zs.at[t])
                emit_inv_b(b, t, AI_ref, Zs.at[t], pad_s)
        return carry

    with _scope("s6_inv"):
        loop(0, 2, inv_body, "inv")
    b_cp(1).start()
    b_cp(2).start()

    for g_ in range(2):
        for p_ in range(16):
            h_ = 2 * p_ + g_
            wo_p[pl.ds((g_ * 16 + p_) * 8, 8), :] = pk16(wo_ref[pl.ds(16 * h_, 16), :].astype(f32))

    def filler(j, t):
        if j == 0 and t == 1:
            emit_epilogue(3, 1, u_ref, dsk_s, pad_s, b_s)
            b_cp(3).start()

    def out_cp(j, half=None):
        if half is None:
            q0, n = al(j * 128, 128), 128
        else:
            q0, n = j * 128 + half * 64, 64
        return pltpu.make_async_copy(a_s.at[pl.ds(q0, n), :], o_h.at[pl.ds(q0, n), pl.ds(0, 512)], sem_out)

    emit_attention(qt_s, k_s, vt_s, wo_p, a_s, oT_a, oT_b, on_s, s_a, s_b, m_a, m_b, lambda j, half: out_cp(j, half).start(), filler)
    with _scope("sA_outwait"):
        pltpu.make_async_copy(o_h, o_h, sem_out).wait()


def scratch_shapes():
    V = pltpu.VMEM
    return [
        V((S_, D_), bf16), V((D_, 3 * D_), bf16), V((D_, D_), bf16), V((L_, D_), bf16),
        V((D_, N_), bf16), V((D_, N_), bf16), V((D_, N_), bf16), V((D_, N_), bf16), V((D_, N_), bf16), V((D_, N_), bf16),
        V((D_,), bf16), V((D_,), bf16),
        V(C_A.shape, u32), V(C_AI.shape, u32),
        V((2, D_ // 2, S_), u32), V((S_ // 2, D_), u32), V((D_ // 2, S_), u32), V((D_ // 2, D_), u32), V((D_ // 2, D_), u32), V((D_ // 2, D_), u32),
        V((128, 128), u32), V((128, 128), u32), V((64, D_), u32),
        V((GS, 256, 128), f32), V((GS, 256, 128), f32), V((GS, 8, 128), f32), V((GS, 8, 128), f32),
        V((S_, D_), bf16), V((L_, D_), bf16),
        V((D_, 128), f32), V((128 * UP + 8, 128), u32), V((128 * UP + 8, 128), u32),
        V((128 * VP + 8, 128), u32), V((128 * VP + 8, 128), u32),
        V((NA * FP + 8, 128), f32), V((4 * TR + 8, 128), f32),
        V((4 * PR, 128), f32), V((ZW, 128), f32), V((2, 2048, 128), u32), V((1, D_), f32),
        pltpu.SemaphoreType.DMA((5,)), pltpu.SemaphoreType.DMA(()),
    ]


@jax.jit
def pallas_concat_heads__sliding_block__ssm_conv_s4__prompt_kernel(
    A_x, A_wqkv, A_wo, B_u, B_A_re, B_A_im, B_B_re, B_B_im, B_C_re, B_C_im, B_log_dt, B_Dskip,
):
    any_spec = pl.BlockSpec(memory_space=pl.ANY)
    out = pl.pallas_call(
        kernel,
        out_shape=jax.ShapeDtypeStruct((S_, 2 * D_), bf16),
        in_specs=[any_spec] * 14,
        out_specs=any_spec,
        scratch_shapes=scratch_shapes(),
        compiler_params=pltpu.CompilerParams(vmem_limit_bytes=112 * 1024 * 1024),
        name="fused",
    )(A_x.reshape(S_, D_), A_wqkv, A_wo, B_u.reshape(L_, D_), B_A_re, B_A_im, B_B_re, B_B_im, B_C_re, B_C_im,
      B_log_dt, B_Dskip, C_A, C_AI)
    return out.reshape(1, S_, 2 * D_)
```

```python
import jax
import jax.numpy as jnp
import numpy as np
from jax import lax
from jax.experimental import pallas as pl
from jax.experimental.pallas import tpu as pltpu

f32, bf16, u32 = jnp.float32, jnp.bfloat16, jnp.uint32
NT = (((1,), (1,)), ((), ()))
NN = (((1,), (0,)), ((), ()))

S_, D_, H_ = 2048, 512, 32
L_, N_ = 2048, 128
NF = 4096
C2 = float(0.25 * np.log2(np.e))
NEG = -1e30
GS = 4
VP, UP, FP = 65, 49, 129
NA = 24
TR = NA * 32
PR = 128 * 17 + 8


def _bf16_round(x):
    x = np.ascontiguousarray(x, dtype=np.float32)
    u = x.view(np.uint32).astype(np.uint64)
    r = ((u + 0x7FFF + ((u >> 16) & 1)) & 0xFFFF0000).astype(np.uint32)
    return r.view(np.float32)


LB = _bf16_round(np.arange(L_, dtype=np.float32)).astype(np.int64)
ALPHAS = list(range(8)) + [256 * m for m in range(1, 9)] + [258, 260, 262, 516, 772]
AIDX = {a: i for i, a in enumerate(ALPHAS)}


def _t_row(t):
    if t < 256:
        return AIDX[t % 8] * 32 + t // 8
    blk = t // 256
    rem = t - 256 * blk
    return AIDX[256 * blk + rem % 8] * 32 + rem // 8


def _pack_rows(x):
    b = _bf16_round(np.asarray(x, dtype=np.float32)).view(np.uint32) >> 16
    return np.ascontiguousarray(b[..., 0::2, :] | (b[..., 1::2, :] << 16)).astype(np.uint32)


def _build_consts():
    k1 = np.arange(128)
    n1 = np.arange(128)
    A = np.zeros((16, 256, 128))
    AI = np.zeros((16, 128, 256))
    p16 = np.array([16 * (j // 16) + (j % 16) // 2 + 8 * (j % 2) for j in range(256)])
    for n2 in range(16):
        th = 2 * np.pi * (k1[:, None] + 0.5) * (16 * n1[None, :] + n2) / NF
        rows = (k1 // 8) * 16 + k1 % 8
        A[n2, rows] = np.cos(th)
        A[n2, rows + 8] = -np.sin(th)
        AI[n2] = (A[n2].T * (2.0 / NF))[:, p16]
    starts = []
    for n2 in range(16):
        st = []
        for v in range(16):
            rows = [_t_row(int(LB[16 * (8 * v + r) + n2])) for r in range(8)]
            assert all(rows[r] == rows[0] + 2 * r for r in range(8))
            st.append(rows[0])
        starts.append(st)
    return _pack_rows(A), _pack_rows(AI), starts


C_A, C_AI, KST = _build_consts()
L_HI = float(np.array([0x3FB8AA00], dtype=np.uint32).view(np.float32)[0])
L_LO = float(1.4426950408889634 - L_HI)


def al(x, m):
    return x if isinstance(x, int) else pl.multiple_of(x, m)


def ld16(w):
    return pltpu.bitcast(w, bf16)


def q16(x):
    return pltpu.bitcast(x.astype(bf16), u32)


def pck(a, b):
    return pltpu.pack_elementwise([a, b], packed_dtype=bf16)


def unp(w, i):
    return pltpu.unpack_elementwise(w, index=i, packed_dtype=bf16, unpacked_dtype=f32)


def pk16(x):
    ws = [pltpu.pack_elementwise([x[16 * i:16 * i + 8], x[16 * i + 8:16 * i + 16]], packed_dtype=bf16)
          for i in range(x.shape[0] // 16)]
    return ws[0] if len(ws) == 1 else jnp.concatenate(ws, axis=0)


def cmul(a, b):
    return (a[0] * b[0] - a[1] * b[1], a[0] * b[1] + a[1] * b[0])


def csq(a):
    return ((a[0] - a[1]) * (a[0] + a[1]), 2.0 * a[0] * a[1])


def sincos(x):
    kf = jnp.floor(x * 0.6366197723675814 + 0.5)
    r = ((x - kf * 1.5703125) - kf * 4.837512969970703125e-4) - kf * 7.54978995489188216e-8
    z = r * r
    s = ((-1.9515295891e-4 * z + 8.3321608736e-3) * z - 1.6666654611e-1) * z * r + r
    c = ((2.443315711809948e-5 * z - 1.388731625493765e-3) * z + 4.166664568298827e-2) * z * z - 0.5 * z + 1.0
    k = kf.astype(jnp.int32)
    swap = (k & 1) == 1
    s2 = jnp.where(swap, c, s)
    c2 = jnp.where(swap, s, c)
    s3 = jnp.where((k & 2) == 2, -s2, s2)
    c3 = jnp.where(((k + 1) & 2) == 2, -c2, c2)
    return s3, c3


def cexp(a, ph):
    e = jnp.exp(a)
    s, c = sincos(ph)
    return (e * c, e * s)


def emit_dt(ldt_ref, dt_s):
    x = ldt_ref[...].astype(f32).reshape(1, D_)
    e = jnp.exp2(x * L_HI)
    e = e + e * ((x * L_LO) * 0.6931471805599453)
    dt = e.astype(bf16).astype(f32)
    for c in range(4):
        dt_s[c * 128:(c + 1) * 128, :] = jnp.broadcast_to(dt[:, c * 128:(c + 1) * 128], (128, 128)).T


def emit_pow(r0, RB, prm, dt_s, Ut, Vt, dep):
    are_ref, aim_ref, bre_ref, bim_ref, cre_ref, cim_ref = prm
    sl = pl.ds(r0, RB)
    c = r0 // 128
    g0 = r0 % 128
    vbase = g0 * VP + c * 16
    ubase = g0 * UP + c * 12
    dtb = dt_s[sl, :]
    dtb = jnp.where(dep[0], dep[1], dtb)
    a = dtb * are_ref[sl, :].astype(f32)
    ph = dtb * aim_ref[sl, :].astype(f32)
    w = cmul((cre_ref[sl, :].astype(f32), cim_ref[sl, :].astype(f32)),
             (dtb * bre_ref[sl, :].astype(f32), dtb * bim_ref[sl, :].astype(f32)))
    l1 = cexp(a, ph)
    l256 = cexp(a * 256.0, ph * 256.0)
    l2 = csq(l1)
    l4 = csq(l2)
    l8 = csq(l4)
    v1 = (l8[0], -l8[1])
    v2 = csq(v1)
    ve, vo = (jnp.ones_like(a), jnp.zeros_like(a)), v1
    for j in range(16):
        for ri in range(2):
            Vt[ri][pl.ds(vbase + j, RB, stride=VP), :] = pck(ve[ri], vo[ri])
        if j < 15:
            ve = v2 if j == 0 else cmul(ve, v2)
            vo = cmul(vo, v2)
    w = (jnp.where(dep[0], vo[0], w[0]), jnp.where(dep[0], vo[0], w[1]))

    def put(j, x, y):
        for ri in range(2):
            Ut[ri][pl.ds(ubase + j, RB, stride=UP), :] = pck(x[ri], y[ri])

    u0 = w
    for j in range(4):
        u1 = cmul(u0, l1)
        put(j, u0, u1)
        if j < 3:
            u0 = cmul(u1, l1)
    u256 = cmul(w, l256)
    u512 = cmul(u256, l256)
    put(4, u256, u512)
    u260 = cmul(u256, l4)
    put(8, cmul(u256, l2), u260)
    put(9, cmul(u260, l2), cmul(u512, l4))
    ua = cmul(u512, l256)
    u772 = cmul(ua, l4)
    put(10, u772, u772)
    put(11, u772, u772)
    ub = cmul(ua, l256)
    put(5, ua, ub)
    ua = cmul(ub, l256)
    ub = cmul(ua, l256)
    put(6, ua, ub)
    ua = cmul(ub, l256)
    ub = cmul(ua, l256)
    put(7, ua, ub)
    return ub[0]


def emit_kgen(g, Ut, Vt, Fs, dep=None):
    lane = lax.broadcasted_iota(jnp.int32, (24, 128), 1)
    Lw = [Ut[ri][pl.ds(g * UP, 48), :] for ri in range(2)]
    if dep is not None:
        Lw[0] = jnp.concatenate([jnp.where(dep[0], pltpu.bitcast(dep[1], u32), Lw[0][0:8]), Lw[0][8:48]], axis=0)
    Lm = jnp.concatenate([pltpu.bitcast(w_, bf16) for w_ in Lw], axis=1)
    Rm = jnp.concatenate([pltpu.bitcast(Vt[ri][pl.ds(g * VP, 64), :], bf16) for ri in range(2)], axis=1)
    out = lax.dot_general(Lm, Rm, NT, preferred_element_type=f32)
    F = jnp.where(lane < 64, jnp.where(lane < 32, out[0:24], out[24:48]),
                  jnp.where(lane < 96, out[48:72], out[72:96]))
    Fs[pl.ds(g, 24, stride=FP), :] = F


def emit_ttrans(idx, Fs, Ts):
    At = Fs[pl.ds(idx * FP, 128), :].T
    for c in range(4):
        Ts[pl.ds(al(c * TR + idx * 32, 8), 32), :] = At[32 * c:32 * c + 32]


def emit_upad(g, u_ref, pad_s):
    for c in range(4):
        w = pltpu.bitcast(u_ref[pl.ds(16 * g, 16), pl.ds(128 * c, 128)], u32)
        for e in range(2):
            pad_s[pl.ds(c * PR + 17 * g + e, 8, stride=2), :] = unp(w, e)


def zrow(c, cc, b):
    return ((c * 4 + cc) * 4 + b) * 256


def emit_f1(b, c, tile, A_ref, Z, zoff):
    zs = [lax.dot_general(ld16(A_ref[4 * a + b]), tile(4 * a + b), NN, preferred_element_type=f32) for a in range(4)]
    for kv in range(16):
        y = _r4([(z[16 * kv:16 * kv + 8], z[16 * kv + 8:16 * kv + 16]) for z in zs], -1)
        for cc in range(4):
            v = _tw(y[cc], b * cc, -1)
            r = zoff + zrow(c, cc, b) + 16 * kv
            Z[pl.ds(al(r, 8), 8), :] = v[0]
            Z[pl.ds(al(r + 8, 8), 8), :] = v[1]


def emit_f1u(b, c, pad_s, A_ref, Z):
    emit_f1(b, c, lambda n2: pad_s[pl.ds(c * PR + n2, 128, stride=17), :], A_ref, Z, ZU)


def emit_f1k(b, c, Ts, A_ref, Z):
    emit_f1(b, c, lambda n2: jnp.concatenate([Ts[pl.ds(c * TR + s0, 8, stride=2), :] for s0 in KST[n2]], axis=0),
            A_ref, Z, ZK)


def _r4(x, sg):
    a0 = (x[0][0] + x[2][0], x[0][1] + x[2][1])
    a1 = (x[0][0] - x[2][0], x[0][1] - x[2][1])
    b0 = (x[1][0] + x[3][0], x[1][1] + x[3][1])
    b1 = (x[1][0] - x[3][0], x[1][1] - x[3][1])
    p = (a1[0] - b1[1], a1[1] + b1[0])
    m = (a1[0] + b1[1], a1[1] - b1[0])
    return [(a0[0] + b0[0], a0[1] + b0[1]), p if sg > 0 else m, (a0[0] - b0[0], a0[1] - b0[1]), m if sg > 0 else p]


def _tw(x, e, sg):
    e = e % 16
    if e == 0:
        return x
    if e == 4:
        return (-x[1], x[0]) if sg > 0 else (x[1], -x[0])
    if e in (2, 6):
        h = float(np.sqrt(0.5))
        if (e == 2) == (sg > 0):
            if e == 2:
                return ((x[0] - x[1]) * h, (x[0] + x[1]) * h)
            return ((x[1] - x[0]) * h, (x[0] + x[1]) * (-h))
        if e == 2:
            return ((x[0] + x[1]) * h, (x[1] - x[0]) * h)
        return ((x[0] + x[1]) * (-h), (x[0] - x[1]) * h)
    c = float(np.cos(2 * np.pi * e / 16))
    s = float(sg * np.sin(2 * np.pi * e / 16))
    return (x[0] * c - x[1] * s, x[0] * s + x[1] * c)


ZU, ZK, ZW = 0, 16384, 32768


def emit_mid(c, cc, kv, Z, z0=0):
    base = zrow(c, cc, 0) + 16 * kv + z0

    def ld(off):
        return [(Z[pl.ds(al(base + off + b * 256, 8), 8), :], Z[pl.ds(al(base + off + b * 256 + 8, 8), 8), :])
                for b in range(4)]

    kh = _r4(ld(ZK), -1)
    uh = _r4(ld(ZU), -1)
    y = _r4([cmul(p, q) for p, q in zip(uh, kh)], +1)
    for b in range(4):
        Z[pl.ds(al(base + ZU + b * 256, 8), 8), :] = y[b][0]
        Z[pl.ds(al(base + ZU + b * 256 + 8, 8), 8), :] = y[b][1]


def emit_inv_a(b, c, Z, zs, Zs):
    IV = 4
    for i, kv in enumerate([h * 8 + j for j in range(8) for h in range(2)]):
        z0 = zs[(i // IV) % len(zs)]
        x = []
        for cc in range(4):
            r = ZU + zrow(c, cc, b) + 16 * kv + z0
            x.append(_tw((Z[pl.ds(al(r, 8), 8), :], Z[pl.ds(al(r + 8, 8), 8), :]), b * cc, +1))
        y = _r4(x, +1)
        for a in range(4):
            Zs[pl.ds((b * 4 + a) * 128 + 8 * kv, 8), :] = pck(y[a][0], y[a][1])


def emit_inv_b(b, t, AI_ref, Zs, pad_s):
    for a in range(4):
        n2 = 4 * a + b
        w = Zs[pl.ds((b * 4 + a) * 128, 128), :]
        y = lax.dot_general(ld16(AI_ref[n2]), ld16(w), NN, preferred_element_type=f32)
        pad_s[pl.ds(t * PR + n2, 128, stride=17), :] = y


def emit_epilogue(c, t, u_ref, dsk_s, pad_s, b_s):
    ls = pl.ds(al(128 * c, 128), 128)
    dk = jnp.broadcast_to(dsk_s[:, ls], (128, 128))
    for g0 in range(0, 128, 8):
        rows = pl.ds(16 * g0, 128)
        y = jnp.concatenate([pad_s[pl.ds(t * PR + 17 * g, 16), :] for g in range(g0, g0 + 8)], axis=0)
        b_s[rows, ls] = (y + u_ref[rows, ls].astype(f32) * dk).astype(bf16)


def emit_attention(qt_s, k_s, vt_s, wo_p, a_s, oT_a, oT_b, on_s, s_a, s_b, m_a, m_b, after_outproj, filler):
    row = lax.broadcasted_iota(jnp.int32, (64, 128), 0)
    lane64 = lax.broadcasted_iota(jnp.int32, (64, 128), 1) & 63
    near_ok = row <= lane64
    lo16 = lax.broadcasted_iota(jnp.int32, (16, 128), 1) < 64
    z8 = jnp.zeros((8, 128), u32)
    z64 = jnp.zeros((64, 128), f32)
    ND = 2
    oTs = (oT_a, oT_b)

    def qk_group(j, par, nch, hg, s_ref, m_ref):
        t0 = al(j * 128, 128)
        wn = al(j * 64 + par * 32, 32)
        ls = pl.ds(hg * 128, 128)
        nmid = min(nch - 1, 3)
        if nch == 5:
            pcs = []
            for i in range(4):
                pcs.append(k_s[pl.ds(al(wn - 128 + 8 * i, 8), 8), ls])
                pcs.append(k_s[pl.ds(al(wn + 8 * i, 8), 8), ls])
            pcs.append(k_s[pl.ds(al(wn - 96, 32), 96), ls])
            Kw = ld16(jnp.concatenate(pcs, axis=0))
        else:
            Kw = ld16(k_s[pl.ds(al(wn - 32 * nmid, 32), 32 * nch), ls])
        for u in range(4):
            p = hg * 4 + u
            qq = qt_s[par, pl.ds(p * 16, 16), pl.ds(t0, 128)]
            W = ld16(jnp.concatenate([z8] * (2 * u) + [qq] + [z8] * (6 - 2 * u), axis=0))
            ST = lax.dot_general(Kw, W, NN, preferred_element_type=f32)
            if nch == 5:
                mrg = jnp.concatenate(
                    [jnp.where(near_ok[16 * i:16 * i + 16], ST[32 * i + 16:32 * i + 32], ST[32 * i:32 * i + 16])
                     for i in range(4)], axis=0)
                mid = ST[128:320]
            else:
                mrg = jnp.where(near_ok, ST[64 * nmid:64 * nmid + 64], NEG)
                mid = ST[0:64 * nmid] if nmid else None
            s_ref[u, 0:64] = mrg
            mx = mrg
            if mid is not None:
                s_ref[u, 64:64 + 64 * nmid] = mid
                for i in range(nmid):
                    mx = jnp.maximum(mx, mid[64 * i:64 * i + 64])
            m_ref[u] = jnp.broadcast_to(jnp.max(mx, axis=0, keepdims=True), (8, 128))

    def pv_group(j, par, nch, hg, s_ref, m_ref):
        nmid = min(nch - 1, 3)
        oT_s = oTs[par]
        for u in range(4):
            p = hg * 4 + u
            m8 = m_ref[u]
            dacc = [None] * ND

            def probs(r0, n):
                x = jnp.exp2((s_ref[u, r0:r0 + n] - jnp.concatenate([m8] * (n // 8), axis=0)) * C2)
                for i in range(n // 8):
                    k = (r0 // 8 + i) % ND
                    dacc[k] = x[8 * i:8 * i + 8] if dacc[k] is None else dacc[k] + x[8 * i:8 * i + 8]
                return x

            def vt(tile, n=128):
                return ld16(vt_s[pl.ds(p * 16, 16), pl.ds(al((j + tile) * 128, 128), n)])

            def pv(v, w):
                return lax.dot_general(v, w.astype(bf16), NN, preferred_element_type=f32)

            pm = probs(0, 64)
            pd = probs(64, 64 * nmid) if nmid else None
            if nch == 5:
                pf = jnp.where(near_ok, 0.0, pm)
                pn = jnp.where(near_ok, pm, 0.0)
                if par == 0:
                    OT = (pv(vt(0, 64), pn) + pv(vt(-2), jnp.concatenate([pf, pd[0:64]], axis=0))
                          + pv(vt(-1), pd[64:192]))
                else:
                    OT = (pv(vt(-2), jnp.concatenate([z64, pf], axis=0)) + pv(vt(-1), pd[0:128])
                          + pv(vt(0), jnp.concatenate([pd[128:192], pn], axis=0)))
            elif nch == 4:
                OT = pv(vt(-1), pd[0:128]) + pv(vt(0), jnp.concatenate([pd[128:192], pm], axis=0))
            elif nch == 3:
                OT = pv(vt(0, 64), pm) + pv(vt(-1), pd[0:128])
            elif nch == 2:
                OT = pv(vt(0), jnp.concatenate([pd[0:64], pm], axis=0))
            else:
                OT = pv(vt(0, 64), pm)
            dl = [x for x in dacc if x is not None]
            while len(dl) > 1:
                dl = [dl[2 * i] + dl[2 * i + 1] for i in range(len(dl) // 2)] + dl[len(dl) // 2 * 2:]
            den = jnp.sum(dl[0], axis=0, keepdims=True)
            o = jnp.where(lo16, OT[0:16], OT[16:32]) * (1.0 / den)
            oT_s[pl.ds(p * 8, 8), :] = pk16(o)

    def otrans(par):
        Tw = pltpu.bitcast(ld16(oTs[par][...]).T, u32)
        on_s[pl.ds(par * 32, 32), pl.ds(0, 256)] = Tw[0:32]
        on_s[pl.ds(par * 32, 32), pl.ds(256, 256)] = Tw[32:64]

    def outproj(j):
        a_s[pl.ds(al(j * 128, 128), 128), :] = jnp.dot(
            ld16(on_s[...]), ld16(wo_p[...]), preferred_element_type=f32).astype(bf16)
        after_outproj(j, None)

    def outproj_half(j, par):
        a_s[pl.ds(j * 128 + par * 64, 64), :] = jnp.dot(
            ld16(on_s[pl.ds(par * 32, 32), :]), ld16(wo_p[...]), preferred_element_type=f32).astype(bf16)
        after_outproj(j, par)

    bufs = [(s_a, m_a), (s_b, m_b)]
    OPG = 2

    def tile_block(j, nchs, nch_next, j_next, has_prev, fill=None):
        for t in range(8):
            par, hg = t // 4, t % 4
            if t + 1 < 8:
                qk_group(j, (t + 1) // 4, nchs[(t + 1) // 4], (t + 1) % 4, *bufs[(t + 1) % 2])
            elif j_next is not None:
                qk_group(j_next, 0, nch_next, 0, *bufs[0])
            pv_group(j, par, nchs[par], hg, *bufs[t % 2])
            if t == 0 and has_prev:
                otrans(1)
            if t == OPG and has_prev:
                outproj(j - 1)
            if t == 4:
                otrans(0)
            if t == 5 and j_next is None:
                outproj_half(j, 0)
            if fill is not None:
                fill(t)

    qk_group(0, 0, 1, 0, *bufs[0])
    tile_block(0, (1, 2), 3, 1, False, lambda t: filler(0, t))
    tile_block(1, (3, 4), 5, 2, True)

    AU = 2

    def body(it, c):
        for t in range(AU):
            j = 2 + it * AU + t
            tile_block(j, (5, 5), 5, j + 1, True)
        return c

    lax.fori_loop(0, 6, body, 0)
    tile_block(14, (5, 5), 5, 15, True)
    tile_block(15, (5, 5), None, None, True)
    otrans(1)
    outproj_half(15, 1)


def kernel(x_h, wqkv_h, wo_h, u_h, are_h, aim_h, bre_h, bim_h, cre_h, cim_h, ldt_h, dsk_h,
           A_h, AI_h,
           o_h,
           x_ref, wqkv_ref, wo_ref, u_ref, are, aim, bre, bim, cre, cim, ldt_ref, dsk_ref,
           A_ref, AI_ref,
           qt_s, k_s, vt_s, wqT, wvT, wo_p, oT_a, oT_b, on_s, s_a, s_b, m_a, m_b, a_s, b_s,
           dt_s, Utr, Uti, Vtr, Vti, Fs, Ts, pad_s, Z, Zs, dsk_s,
           sem_in, sem_out):
    Ut = (Utr, Uti)
    Vt = (Vtr, Vti)
    prm = (are, aim, bre, bim, cre, cim)
    TB = 256
    NB = S_ // TB
    cps = {}
    groups = (("wk", "x0"), ("x1", "x2"), ("wq", "wv", "x3", "ldt"),
              ("x4", "x5", "x6", "x7", "p0", "p1", "p2", "p3", "p4", "p5"),
              ("u", "A", "AI", "dsk", "wo"))
    sem_of = {n: i for i, g in enumerate(groups) for n in g}

    def mk(name, src, dst):
        cps[name] = pltpu.make_async_copy(src, dst, sem_in.at[sem_of[name]])

    mk("wk", wqkv_h.at[:, pl.ds(512, 512)], wqkv_ref.at[:, pl.ds(512, 512)])
    mk("wq", wqkv_h.at[:, pl.ds(0, 512)], wqkv_ref.at[:, pl.ds(0, 512)])
    mk("wv", wqkv_h.at[:, pl.ds(1024, 512)], wqkv_ref.at[:, pl.ds(1024, 512)])
    for i in range(NB):
        mk("x%d" % i, x_h.at[pl.ds(i * TB, TB), :], x_ref.at[pl.ds(i * TB, TB), :])
    mk("ldt", ldt_h, ldt_ref)
    for i, (s, d) in enumerate(zip((are_h, aim_h, bre_h, bim_h, cre_h, cim_h), prm)):
        mk("p%d" % i, s, d)
    mk("u", u_h, u_ref)
    mk("A", A_h, A_ref)
    mk("AI", AI_h, AI_ref)
    mk("dsk", dsk_h, dsk_ref)
    mk("wo", wo_h, wo_ref)

    def start(*names):
        for n in names:
            cps[n].start()

    def kproj(r0):
        k_s[pl.ds(al(r0 // 2, TB // 2), TB // 2), :] = q16(
            jnp.dot(x_ref[pl.ds(r0, TB), :], wqkv_ref[:, 512:1024], preferred_element_type=f32))

    def qproj(r0):
        xb = x_ref[pl.ds(r0, TB), :]
        qw = q16(lax.dot_general(ld16(wqT[...]), xb, NT, preferred_element_type=f32))
        lo = lax.broadcasted_iota(jnp.int32, (8, 128), 1) < 64
        z = jnp.zeros((8, 128), u32)
        for c in range(TB // 128):
            nat = qw[:, 128 * c:128 * c + 128]
            rol = pltpu.roll(nat, 64, 1)
            for h in range(H_):
                a_, b_ = nat[8 * h:8 * h + 8], rol[8 * h:8 * h + 8]
                dst = (pl.ds(8 * h, 8), pl.ds(al(r0 + 128 * c, 128), 128))
                if h % 2 == 0:
                    qt_s[(0,) + dst] = jnp.where(lo, a_, z)
                    qt_s[(1,) + dst] = jnp.where(lo, b_, z)
                else:
                    qt_s[(0,) + dst] = jnp.where(lo, z, b_)
                    qt_s[(1,) + dst] = jnp.where(lo, z, a_)

    def vproj(r0):
        xb = x_ref[pl.ds(r0, TB), :]
        vt_s[:, pl.ds(r0, TB)] = q16(lax.dot_general(ld16(wvT[...]), xb, NT, preferred_element_type=f32))

    def qvproj(*r0s):
        for r0 in r0s:
            qproj(r0)
            vproj(r0)

    pow_state = {}

    def pow_gblock(gb):
        never = dt_s[pl.ds(0, 8), :] < -1.0
        last = pow_state.get("last")
        if last is None:
            last = dt_s[pl.ds(0, 8), :]
        for c in range(4):
            last = emit_pow(128 * c + 8 * gb, 8, prm, dt_s, Ut, Vt, (never, last))
        pow_state["last"] = last

    def waitn(*names):
        for n in names:
            cps[n].wait()

    start("wk", "x0", "x1", "x2", "wq", "wv", "x3", "ldt", "x4", "x5", "p0", "p1", "p2", "p3", "p4", "p5", "x6", "x7")
    waitn("wk", "x0")
    kproj(0)
    waitn("x1", "x2")
    start("u", "A")
    kproj(TB)
    kproj(2 * TB)
    waitn("wq", "wv", "x3", "ldt")
    start("AI", "dsk", "wo")
    wqT[...] = pltpu.bitcast(wqkv_ref[:, 0:512].T, u32)
    wvT[...] = pltpu.bitcast(wqkv_ref[:, 1024:1536].T, u32)
    kproj(3 * TB)
    emit_dt(ldt_ref, dt_s)
    qvproj(0, TB)

    PB1 = 11
    waitn("x4", "x5", "x6", "x7", "p0", "p1", "p2", "p3", "p4", "p5")
    for gb in range(PB1):
        pow_gblock(gb)
    qvproj(2 * TB, 3 * TB)
    for i in (4, 5, 6, 7):
        kproj(i * TB)
    pow_state.clear()

    waitn("u", "A", "AI", "dsk", "wo")
    dsk_s[...] = dsk_ref[...].astype(f32).reshape(1, D_)
    PST = 10
    for g in range(128):
        if g % PST == 0 and PB1 + g // PST < 16:
            pow_gblock(PB1 + g // PST)
        emit_kgen(g, Ut, Vt, Fs, (dt_s[pl.ds(0, 8), :] < -1.0, pow_state["last"]) if g == 75 else None)
        emit_upad(g, u_ref, pad_s)
    for i in range(16):
        emit_f1u(i % 4, i // 4, pad_s, A_ref, Z)
        for idx in range(i * 21 // 12, min(21, (i + 1) * 21 // 12)):
            emit_ttrans(idx, Fs, Ts)
    for c in range(4):
        for b in range(4):
            emit_f1k(b, c, Ts, A_ref, Z)

    def b_cp(c):
        l0 = al(128 * c, 128)
        return pltpu.make_async_copy(b_s.at[:, pl.ds(l0, 128)], o_h.at[:, pl.ds(al(512 + l0, 128), 128)], sem_out)

    def zeros_chain(c):
        return [((c * (2 * i + 3)) >> 12) * 8 for i in range(3)]

    def mid_c(c):
        zs = zeros_chain(c)
        for i in range(64):
            emit_mid(c, i // 16, i % 16, Z, zs[i % len(zs)])

    def proj_body3(it, c):
        qvproj(al((4 + it) * TB, TB))
        mid_c(it)
        return c

    lax.fori_loop(0, 4, proj_body3, 0)

    def inv_body(it, carry):
        @pl.when(it > 0)
        def _():
            b_cp(0).start()

        zs = zeros_chain(it)
        for t in range(2):
            c = 2 * it + t
            emit_epilogue(jnp.maximum(c - 1, 0), 1 - t, u_ref, dsk_s, pad_s, b_s)
            for b in range(4):
                emit_inv_a(b, c, Z, zs, Zs.at[t])
                emit_inv_b(b, t, AI_ref, Zs.at[t], pad_s)
        return carry

    lax.fori_loop(0, 2, inv_body, 0)
    b_cp(1).start()
    b_cp(2).start()

    for g_ in range(2):
        for p_ in range(16):
            h_ = 2 * p_ + g_
            wo_p[pl.ds((g_ * 16 + p_) * 8, 8), :] = pk16(wo_ref[pl.ds(16 * h_, 16), :].astype(f32))

    def filler(j, t):
        if j == 0 and t == 1:
            emit_epilogue(3, 1, u_ref, dsk_s, pad_s, b_s)
            b_cp(3).start()

    def out_cp(j, half=None):
        if half is None:
            q0, n = al(j * 128, 128), 128
        else:
            q0, n = j * 128 + half * 64, 64
        return pltpu.make_async_copy(a_s.at[pl.ds(q0, n), :], o_h.at[pl.ds(q0, n), pl.ds(0, 512)], sem_out)

    emit_attention(qt_s, k_s, vt_s, wo_p, a_s, oT_a, oT_b, on_s, s_a, s_b, m_a, m_b, lambda j, half: out_cp(j, half).start(), filler)
    pltpu.make_async_copy(o_h, o_h, sem_out).wait()


def scratch_shapes():
    V = pltpu.VMEM
    return [
        V((S_, D_), bf16), V((D_, 3 * D_), bf16), V((D_, D_), bf16), V((L_, D_), bf16),
        V((D_, N_), bf16), V((D_, N_), bf16), V((D_, N_), bf16), V((D_, N_), bf16), V((D_, N_), bf16), V((D_, N_), bf16),
        V((D_,), bf16), V((D_,), bf16),
        V(C_A.shape, u32), V(C_AI.shape, u32),
        V((2, D_ // 2, S_), u32), V((S_ // 2, D_), u32), V((D_ // 2, S_), u32), V((D_ // 2, D_), u32), V((D_ // 2, D_), u32), V((D_ // 2, D_), u32),
        V((128, 128), u32), V((128, 128), u32), V((64, D_), u32),
        V((GS, 256, 128), f32), V((GS, 256, 128), f32), V((GS, 8, 128), f32), V((GS, 8, 128), f32),
        V((S_, D_), bf16), V((L_, D_), bf16),
        V((D_, 128), f32), V((128 * UP + 8, 128), u32), V((128 * UP + 8, 128), u32),
        V((128 * VP + 8, 128), u32), V((128 * VP + 8, 128), u32),
        V((NA * FP + 8, 128), f32), V((4 * TR + 8, 128), f32),
        V((4 * PR, 128), f32), V((ZW, 128), f32), V((2, 2048, 128), u32), V((1, D_), f32),
        pltpu.SemaphoreType.DMA((5,)), pltpu.SemaphoreType.DMA(()),
    ]


@jax.jit
def pallas_concat_heads__sliding_block__ssm_conv_s4__prompt_kernel(
    A_x, A_wqkv, A_wo, B_u, B_A_re, B_A_im, B_B_re, B_B_im, B_C_re, B_C_im, B_log_dt, B_Dskip,
):
    any_spec = pl.BlockSpec(memory_space=pl.ANY)
    out = pl.pallas_call(
        kernel,
        out_shape=jax.ShapeDtypeStruct((S_, 2 * D_), bf16),
        in_specs=[any_spec] * 14,
        out_specs=any_spec,
        scratch_shapes=scratch_shapes(),
        compiler_params=pltpu.CompilerParams(vmem_limit_bytes=112 * 1024 * 1024),
        name="fused",
    )(A_x.reshape(S_, D_), A_wqkv, A_wo, B_u.reshape(L_, D_), B_A_re, B_A_im, B_B_re, B_B_im, B_C_re, B_C_im,
      B_log_dt, B_Dskip, C_A, C_AI)
    return out.reshape(1, S_, 2 * D_)
```
